```python
import jax
import jax.numpy as jnp

def _softmax(x, axis=-1):
    return jax.nn.softmax(x, axis=axis)

def _gelu(x):
    return jax.nn.gelu(x, approximate=True)

def _silu(x):
    return jax.nn.silu(x)

def _sigmoid(x):
    return jax.nn.sigmoid(x)

def _layernorm(x, axis=-1, eps=1e-05):
    m = jnp.mean(x, axis=axis, keepdims=True)
    v = jnp.var(x, axis=axis, keepdims=True)
    return (x - m) / jnp.sqrt(v + eps)

def _scatter_add(tgt, idx, src, axis=0):
    return tgt.at[idx].add(src)

def _segment_sum(src, seg, n):
    return jax.ops.segment_sum(src, seg, n)

class _Rng:

    def __init__(self, key):
        self._k = key

    def _next(self):
        self._k, sub = jax.random.split(self._k)
        return sub

    def normal(self, shape):
        return jax.random.normal(self._next(), shape, dtype=jnp.bfloat16)

    def randint(self, lo, hi, shape):
        return jax.random.randint(self._next(), shape, lo, hi, dtype=jnp.int32)

    def uniform(self, shape, lo=0.0, hi=1.0):
        return jax.random.uniform(self._next(), shape, jnp.bfloat16, lo, hi)

    def permutation(self, n):
        return jax.random.permutation(self._next(), n)
kernel_name = 'adaLN_cond__sliding_block_cached__glu_gated_glu__decode'

def setup_inputs():
    _rng = _Rng(jax.random.key(int.from_bytes(__import__("os").urandom(4), "little")))
    _w = lambda a: (lambda t: t.astype(jnp.bfloat16) if jnp.issubdtype(t.dtype, jnp.floating) else t)(jnp.asarray(a))

    def _A_setup():
        B, Sq, D = (8, 1, 512)
        Hq, Hkv, Sk, Dh = (32, 32, 4096, 128)
        assert Hq % Hkv == 0, (Hq, Hkv)
        return {'x': _w((lambda *s: _rng.normal(s) * 0.05)(B, Sq, D)), 'k_cache': _w((lambda *s: _rng.normal(s) * 0.05)(B, Hkv, Sk, Dh)), 'v_cache': _w((lambda *s: _rng.normal(s) * 0.05)(B, Hkv, Sk, Dh)), 'wq': _w((lambda *s: _rng.normal(s) * 0.05)(D, Hq * Dh) * D ** (-0.5)), 'wo': _w((lambda *s: _rng.normal(s) * 0.05)(Hq * Dh, D) * (Hq * Dh) ** (-0.5))}
    _A_in = _A_setup()

    def _B_setup():
        B, S, D, F = (8, 1, 512, 1376)
        return {'x': _w((lambda *s: _rng.normal(s) * 0.05)(B, S, D)), 'w_gate': _w((lambda *s: _rng.normal(s) * 0.05)(D, F)), 'w_up': _w((lambda *s: _rng.normal(s) * 0.05)(D, F)), 'w_down': _w((lambda *s: _rng.normal(s) * 0.05)(F, D))}
    _B_in = _B_setup()
    return {'A_x': _A_in['x'], 'A_k_cache': _A_in['k_cache'], 'A_v_cache': _A_in['v_cache'], 'A_wq': _A_in['wq'], 'A_wo': _A_in['wo'], 'B_x': _B_in['x'], 'B_w_gate': _B_in['w_gate'], 'B_w_up': _B_in['w_up'], 'B_w_down': _B_in['w_down'], 'c': _w((lambda *s: _rng.normal(s) * 0.05)(8, 512)), 'w_mod': _w((lambda *s: _rng.normal(s) * 0.05)(512, 6 * 512) * 512 ** (-0.5))}

def reference(A_x, A_k_cache, A_v_cache, A_wq, A_wo, B_x, B_w_gate, B_w_up, B_w_down, c, w_mod):

    def _A_ref(x, k_cache, v_cache, wq, wo):
        B, Sq, D = x.shape
        Hq, Dh = (32, 128)
        Hkv, Sk = (k_cache.shape[1], k_cache.shape[2])
        W = min(4096, max(256, Sk // 4))
        rep = Hq // Hkv
        q = (lambda x, *d: x.transpose(*d))((x @ wq).reshape(B, Sq, Hq, Dh), 0, 2, 1, 3)
        k = jnp.repeat(k_cache[:, :, Sk - W:, :], rep, axis=1)
        v = jnp.repeat(v_cache[:, :, Sk - W:, :], rep, axis=1)
        scores = jnp.einsum('bhqd,bhkd->bhqk', q, k) * Dh ** (-0.5)
        p = _softmax(scores, axis=-1)
        o = jnp.einsum('bhqk,bhkd->bhqd', p, v)
        return (lambda x, *d: x.transpose(*d))(o, 0, 2, 1, 3).reshape(B, Sq, Hq * Dh) @ wo

    def _B_ref(x, w_gate, w_up, w_down):
        g = jnp.einsum('bsd,df->bsf', x, w_gate)
        u = jnp.einsum('bsd,df->bsf', x, w_up)
        h = _sigmoid(g) * u
        return jnp.einsum('bsf,fd->bsd', h, w_down)
    x = A_x
    mod = (_silu(c) @ w_mod).reshape(c.shape[0], 6, 1, -1)
    sa, ca, ga, sb, cb, gb = (mod[:, 0].copy(), mod[:, 1].copy(), mod[:, 2].copy(), mod[:, 3].copy(), mod[:, 4].copy(), mod[:, 5].copy())
    h = _layernorm(x, axis=-1) * (1 + ca) + sa
    x = x + ga * _A_ref(h, A_k_cache, A_v_cache, A_wq, A_wo)
    h = _layernorm(x, axis=-1) * (1 + cb) + sb
    x = x + gb * _B_ref(h, B_w_gate, B_w_up, B_w_down)
    return x
```

```python
import functools

import jax
import jax.numpy as jnp
import jax.experimental.pallas as pl
import jax.experimental.pallas.tpu as pltpu

_NT = (((1,), (1,)), ((), ()))
_EPS = 1e-5


def _layernorm(x):
    m = jnp.mean(x, axis=-1, keepdims=True)
    xc = x - m
    v = jnp.mean(xc * xc, axis=-1, keepdims=True)
    return xc * jax.lax.rsqrt(v + _EPS)


def _kernel(x_hbm, k_hbm, v_hbm, wq_hbm, wo_hbm, wg_hbm, wu_hbm, wd_hbm, c_hbm, wm_hbm,
            o_ref,
            x_v, c_v, wm_v, wq_v, wo_v, wg_v, wu_v, wd_v, kbuf, vbuf, q_v, att_v, wsem, kvsem,
            *, nbuf, W):
    B, H, S, Dh = k_hbm.shape
    D = x_v.shape[-1]
    bf16 = jnp.bfloat16
    f32 = jnp.float32

    def wcopy(i, src, dst):
        return pltpu.make_async_copy(src, dst, wsem.at[i])

    cp_c = wcopy(0, c_hbm, c_v)
    cp_x = wcopy(1, x_hbm, x_v)
    cp_wm = wcopy(2, wm_hbm, wm_v)
    cp_wq = wcopy(3, wq_hbm, wq_v)
    cp_wo = wcopy(4, wo_hbm, wo_v)
    cp_wg = wcopy(5, wg_hbm, wg_v)
    cp_wu = wcopy(6, wu_hbm, wu_v)
    cp_wd = wcopy(7, wd_hbm, wd_v)

    def kv_copy(a, h, slot):
        src, dst = ((k_hbm, kbuf), (v_hbm, vbuf))[a]
        return pltpu.make_async_copy(src.at[:, h, pl.ds(S - W, W), :], dst.at[slot], kvsem.at[a, slot])

    cp_c.start()
    cp_x.start()
    cp_wm.start()
    cp_wq.start()
    for i in range(nbuf):
        kv_copy(0, i, i).start()
        kv_copy(1, i, i).start()

    cp_c.wait()
    cp_x.wait()
    cp_wm.wait()
    c = c_v[...].astype(f32)
    sc = (c * jax.nn.sigmoid(c)).astype(bf16)
    mod = jnp.dot(sc, wm_v[...], preferred_element_type=f32)
    sa, ca, ga, sb, cb, gb = [mod[:, i * D:(i + 1) * D] for i in range(6)]
    x = x_v[...].astype(f32)
    h1 = (_layernorm(x) * (1.0 + ca) + sa).astype(bf16)
    cp_wq.wait()
    q = jnp.dot(h1, wq_v[...], preferred_element_type=f32) * (Dh ** -0.5)
    for h in range(H):
        q_v[h] = q[:, h * Dh:(h + 1) * Dh]

    row = jax.lax.broadcasted_iota(jnp.int32, (B, W), 0)

    def body(h, carry):
        slot = h % nbuf
        qh = q_v[h].astype(bf16)
        kv_copy(0, h, slot).wait()
        s = jnp.zeros((B, W), f32)
        for b in range(B):
            sb_ = jax.lax.dot_general(qh, kbuf[slot, b], _NT, preferred_element_type=f32)
            s = jnp.where(row == b, sb_, s)
        m = jnp.max(s, axis=-1, keepdims=True)
        p = jnp.exp(s - m)
        l = jnp.sum(p, axis=-1, keepdims=True)
        kv_copy(1, h, slot).wait()
        o = jnp.zeros((B, Dh), f32)
        for b in range(B):
            pb = jnp.where(row == b, p, 0.0).astype(bf16)
            o = o + jnp.dot(pb, vbuf[slot, b], preferred_element_type=f32)
        att_v[h] = o / l

        @pl.when(h + nbuf < H)
        def _():
            kv_copy(0, h + nbuf, slot).start()
            kv_copy(1, h + nbuf, slot).start()

        @pl.when(h + nbuf == H)
        def _():
            cp_wo.start()
            cp_wg.start()
            cp_wu.start()
            cp_wd.start()

        return carry

    jax.lax.fori_loop(0, H, body, 0)

    att = jnp.concatenate([att_v[h] for h in range(H)], axis=-1).astype(bf16)
    cp_wo.wait()
    a_out = jnp.dot(att, wo_v[...], preferred_element_type=f32)
    x1 = x + ga * a_out
    h2 = (_layernorm(x1) * (1.0 + cb) + sb).astype(bf16)
    cp_wg.wait()
    g = jax.lax.dot_general(h2, wg_v[...], _NT, preferred_element_type=f32)
    cp_wu.wait()
    u = jax.lax.dot_general(h2, wu_v[...], _NT, preferred_element_type=f32)
    hh = (jax.nn.sigmoid(g) * u).astype(bf16)
    cp_wd.wait()
    f = jnp.dot(hh, wd_v[...], preferred_element_type=f32)
    o_ref[...] = (x1 + gb * f).astype(o_ref.dtype)


@jax.jit
def pallas_adaLN_cond__sliding_block_cached__glu_gated_glu__decode_kernel(
    A_x: jax.Array,
    A_k_cache: jax.Array,
    A_v_cache: jax.Array,
    A_wq: jax.Array,
    A_wo: jax.Array,
    B_x: jax.Array,
    B_w_gate: jax.Array,
    B_w_up: jax.Array,
    B_w_down: jax.Array,
    c: jax.Array,
    w_mod: jax.Array,
):
    B, Sq, D = A_x.shape
    _, H, S, Dh = A_k_cache.shape
    F = B_w_down.shape[0]
    W = min(4096, max(256, S // 4))
    nbuf = 4
    bf16 = jnp.bfloat16
    any_spec = pl.BlockSpec(memory_space=pl.ANY)
    out = pl.pallas_call(
        functools.partial(_kernel, nbuf=nbuf, W=W),
        in_specs=[any_spec] * 10,
        out_specs=pl.BlockSpec(memory_space=pltpu.VMEM),
        out_shape=jax.ShapeDtypeStruct((B, D), A_x.dtype),
        scratch_shapes=[
            pltpu.VMEM((B, D), bf16),
            pltpu.VMEM((B, D), bf16),
            pltpu.VMEM(w_mod.shape, bf16),
            pltpu.VMEM(A_wq.shape, bf16),
            pltpu.VMEM(A_wo.shape, bf16),
            pltpu.VMEM((F, D), bf16),
            pltpu.VMEM((F, D), bf16),
            pltpu.VMEM((F, D), bf16),
            pltpu.VMEM((nbuf, B, W, Dh), bf16),
            pltpu.VMEM((nbuf, B, W, Dh), bf16),
            pltpu.VMEM((H, B, Dh), jnp.float32),
            pltpu.VMEM((H, B, Dh), jnp.float32),
            pltpu.SemaphoreType.DMA((8,)),
            pltpu.SemaphoreType.DMA((2, nbuf)),
        ],
        compiler_params=pltpu.CompilerParams(vmem_limit_bytes=100 * 1024 * 1024),
    )(A_x.reshape(B, D), A_k_cache, A_v_cache, A_wq, A_wo, B_w_gate.T, B_w_up.T, B_w_down, c, w_mod)
    return out.reshape(B, Sq, D)
```

```python
import functools

import jax
import jax.numpy as jnp
import jax.experimental.pallas as pl
import jax.experimental.pallas.tpu as pltpu

_NT = (((1,), (1,)), ((), ()))
_EPS = 1e-5
_F32 = jnp.float32
_BF16 = jnp.bfloat16


def _layernorm(x):
    m = jnp.mean(x, axis=-1, keepdims=True)
    xc = x - m
    v = jnp.mean(xc * xc, axis=-1, keepdims=True)
    return xc * jax.lax.rsqrt(v + _EPS)


class _Piece:
    def __init__(self, parts, whole, sem):
        self.parts, self.whole, self.sem = parts, whole, sem

    def start(self):
        for src, dst, prio in self.parts:
            pltpu.make_async_copy(src, dst, self.sem).start(priority=prio)

    def wait(self):
        pltpu.make_async_copy(self.whole, self.whole, self.sem).wait()


def _row_piece(src, dst, n, n0, sem):
    n0 = min(n0, n)
    parts = []
    if n0 > 0:
        parts.append((src.at[pl.ds(0, n0)], dst.at[pl.ds(0, n0)], 0))
    if n0 < n:
        parts.append((src.at[pl.ds(n0, n - n0)], dst.at[pl.ds(n0, n - n0)], 1))
    return _Piece(parts, dst, sem)


def _col_piece(src, dst, c0, sem):
    n = src.shape[-1]
    parts = [(src.at[:, pl.ds(0, c0)], dst.at[:, pl.ds(0, c0)], 0),
             (src.at[:, pl.ds(c0, n - c0)], dst.at[:, pl.ds(c0, n - c0)], 1)]
    return _Piece(parts, dst, sem)


def _kernel(x_hbm, k_hbm, v_hbm, wq_hbm, wo_hbm, wg_hbm, wu_hbm, wd_hbm, c_hbm, wm_hbm,
            o_ref,
            x_v, c_v, wm_v, wq_v, wo_v, wg_v, wu_v, wd_v, kbuf, vbuf, q_v, sems,
            *, W, rows, crows, r0, look, wrow0):
    B, H, S, Dh = k_hbm.shape
    D = x_v.shape[-1]
    F = wd_v.shape[0]
    nsem = sems.shape[0]
    npr = W // rows

    counter = [0]

    def next_sem():
        i = counter[0] % nsem
        counter[0] += 1
        return sems.at[i]

    pro = [_Piece([(c_hbm, c_v, 0)], c_v, next_sem()),
           _Piece([(x_hbm, x_v, 0)], x_v, next_sem())]
    mrows = 16
    nm = D // mrows
    morder = [(i % 2) * (nm // 2) + i // 2 for i in range(nm)]
    for i in morder:
        sl = pl.ds(i * mrows, mrows)
        pro.append(_col_piece(wm_hbm.at[sl], wm_v.at[sl], 768, next_sem()))
    n_mod = len(pro)
    for i in morder:
        sl = pl.ds(i * mrows, mrows)
        pro.append(_col_piece(wq_hbm.at[sl], wq_v.at[sl], 1024, next_sem()))

    n_head = 2 * B * npr + 1
    assert nsem == n_head and look + crows // rows <= n_head
    sem0 = counter[0]

    bgroups = [(b, b + B // 2) for b in range(B // 2)]
    br_order = [(b, r) for g in bgroups for r in range(npr) for b in g]

    def head_pieces(h):
        out = []
        for a, (src, dst) in enumerate(((k_hbm, kbuf), (v_hbm, vbuf))):
            for b, r in br_order:
                if True:
                    out.append(_row_piece(src.at[b, h, pl.ds(S - W + r * rows, rows)],
                                          dst.at[b, pl.ds(r * rows, rows)], rows, r0,
                                          sems.at[(sem0 + len(out)) % nsem]))
        ho = h * Dh
        if not isinstance(h, int):
            ho = pl.multiple_of(ho, Dh)
        out.append(_row_piece(wo_hbm.at[pl.ds(ho, Dh)], wo_v, Dh, wrow0,
                              sems.at[(sem0 + len(out)) % nsem]))
        return out

    fchunks = [(f, min(128, F - f)) for f in range(0, F, 128)]
    epi = []
    for f, n in fchunks:
        for src, dst in ((wg_hbm, wg_v), (wu_hbm, wu_v), (wd_hbm, wd_v)):
            epi.append(_row_piece(src.at[pl.ds(f, n)], dst.at[pl.ds(f, n)], n, wrow0, next_sem()))

    def advance(cur, nxt, j):
        cur[j].wait()
        t = j + look
        if t < len(cur):
            cur[t].start()
        elif t - len(cur) < len(nxt):
            nxt[t - len(cur)].start()

    head0 = head_pieces(0)
    for p in pro[:look]:
        p.start()
    for j in range(n_mod):
        advance(pro, head0, j)
    c = c_v[...].astype(_F32)
    sc = (c * jax.nn.sigmoid(c)).astype(_BF16)
    mod = jnp.dot(sc, wm_v[...], preferred_element_type=_F32)
    sa, ca, ga, sb, cb, gb = [mod[:, i * D:(i + 1) * D] for i in range(6)]
    x = x_v[...].astype(_F32)
    h1 = (_layernorm(x) * (1.0 + ca) + sa).astype(_BF16)
    for j in range(n_mod, len(pro)):
        advance(pro, head0, j)
    q = jnp.dot(h1, wq_v[...], preferred_element_type=_F32) * (Dh ** -0.5)
    for h in range(H):
        q_v[h] = q[:, h * Dh:(h + 1) * Dh]

    row = jax.lax.broadcasted_iota(jnp.int32, (B, rows), 0)
    ppc = crows // rows

    def head(h, nxt, a_out):
        cur = head_pieces(h)
        qh = q_v[h].astype(_BF16)
        s = [jnp.zeros((B, rows), _F32) for _ in range(npr)]
        nk = len(br_order)
        for j0 in range(0, nk, ppc):
            for j in range(j0, j0 + ppc):
                advance(cur, nxt, j)
            for b, r in br_order[j0:j0 + ppc]:
                sp = jax.lax.dot_general(qh, kbuf[b, pl.ds(r * rows, rows), :], _NT,
                                         preferred_element_type=_F32)
                s[r] = jnp.where(row == b, sp, s[r])
        m = functools.reduce(jnp.maximum, s)
        m = jnp.max(m, axis=-1, keepdims=True)
        p = [jnp.exp(t - m) for t in s]
        l = jnp.sum(functools.reduce(jnp.add, p), axis=-1, keepdims=True)
        o = jnp.zeros((B, Dh), _F32)
        for j0 in range(0, nk, ppc):
            for j in range(j0, j0 + ppc):
                advance(cur, nxt, nk + j)
            for b, r in br_order[j0:j0 + ppc]:
                pb = jnp.where(row == b, p[r], 0.0).astype(_BF16)
                o = o + jnp.dot(pb, vbuf[b, pl.ds(r * rows, rows), :], preferred_element_type=_F32)
        j = 2 * nk
        att = (o / l).astype(_BF16)
        advance(cur, nxt, j)
        return a_out + jnp.dot(att, wo_v[...], preferred_element_type=_F32)

    a_out = jax.lax.fori_loop(0, H - 1, lambda h, acc: head(h, head_pieces(h + 1), acc),
                              jnp.zeros((B, D), _F32))
    a_out = head(H - 1, epi, a_out)

    x1 = x + ga * a_out
    h2 = (_layernorm(x1) * (1.0 + cb) + sb).astype(_BF16)
    acc = jnp.zeros((B, D), _F32)
    for i, (f, n) in enumerate(fchunks):
        advance(epi, [], 3 * i)
        g = jax.lax.dot_general(h2, wg_v[pl.ds(f, n), :], _NT, preferred_element_type=_F32)
        advance(epi, [], 3 * i + 1)
        u = jax.lax.dot_general(h2, wu_v[pl.ds(f, n), :], _NT, preferred_element_type=_F32)
        hh = (jax.nn.sigmoid(g) * u).astype(_BF16)
        advance(epi, [], 3 * i + 2)
        acc = acc + jnp.dot(hh, wd_v[pl.ds(f, n), :], preferred_element_type=_F32)
    o_ref[...] = (x1 + gb * acc).astype(o_ref.dtype)


def _forward(A_x, A_k_cache, A_v_cache, A_wq, A_wo, B_w_gate, B_w_up, B_w_down, c, w_mod,
             rows=512, crows=1024, r0=192, look=12, wrow0=32, nobounds=True):
    B, Sq, D = A_x.shape
    _, H, S, Dh = A_k_cache.shape
    F = B_w_down.shape[0]
    W = min(4096, max(256, S // 4))
    nsem = 2 * B * (W // rows) + 1
    any_spec = pl.BlockSpec(memory_space=pl.ANY)
    out = pl.pallas_call(
        functools.partial(_kernel, W=W, rows=rows, crows=crows, r0=r0, look=look, wrow0=wrow0),
        in_specs=[any_spec] * 10,
        out_specs=pl.BlockSpec(memory_space=pltpu.VMEM),
        out_shape=jax.ShapeDtypeStruct((B, D), A_x.dtype),
        scratch_shapes=[
            pltpu.VMEM((B, D), _BF16),
            pltpu.VMEM((B, D), _BF16),
            pltpu.VMEM(w_mod.shape, _BF16),
            pltpu.VMEM(A_wq.shape, _BF16),
            pltpu.VMEM((Dh, D), _BF16),
            pltpu.VMEM((F, D), _BF16),
            pltpu.VMEM((F, D), _BF16),
            pltpu.VMEM((F, D), _BF16),
            pltpu.VMEM((B, W, Dh), _BF16),
            pltpu.VMEM((B, W, Dh), _BF16),
            pltpu.VMEM((H, B, Dh), _F32),
            pltpu.SemaphoreType.DMA((nsem,)),
        ],
        compiler_params=pltpu.CompilerParams(vmem_limit_bytes=64 * 1024 * 1024,
                                             disable_bounds_checks=nobounds),
    )(A_x.reshape(B, D), A_k_cache, A_v_cache, A_wq, A_wo, B_w_gate.T, B_w_up.T, B_w_down, c, w_mod)
    return out.reshape(B, Sq, D)


@jax.jit
def pallas_adaLN_cond__sliding_block_cached__glu_gated_glu__decode_kernel(
    A_x: jax.Array,
    A_k_cache: jax.Array,
    A_v_cache: jax.Array,
    A_wq: jax.Array,
    A_wo: jax.Array,
    B_x: jax.Array,
    B_w_gate: jax.Array,
    B_w_up: jax.Array,
    B_w_down: jax.Array,
    c: jax.Array,
    w_mod: jax.Array,
):
    del B_x
    return _forward(A_x, A_k_cache, A_v_cache, A_wq, A_wo, B_w_gate, B_w_up, B_w_down, c, w_mod)
```

```python
import functools

import jax
import jax.numpy as jnp
import jax.experimental.pallas as pl
import jax.experimental.pallas.tpu as pltpu

_NT = (((1,), (1,)), ((), ()))
_EPS = 1e-5
_F32 = jnp.float32
_BF16 = jnp.bfloat16
_G = 8


def _layernorm(x):
    m = jnp.mean(x, axis=-1, keepdims=True)
    xc = x - m
    v = jnp.mean(xc * xc, axis=-1, keepdims=True)
    return xc * jax.lax.rsqrt(v + _EPS)


class _Piece:
    def __init__(self, src, dst, n0, sem):
        n = dst.shape[0]
        n0 = min(n0, n)
        self.parts = []
        if n0 > 0:
            self.parts.append((src.at[pl.ds(0, n0)], dst.at[pl.ds(0, n0)], 0))
        if n0 < n:
            self.parts.append((src.at[pl.ds(n0, n - n0)], dst.at[pl.ds(n0, n - n0)], 1))
        self.whole, self.sem = dst, sem

    def start(self):
        for src, dst, prio in self.parts:
            pltpu.make_async_copy(src, dst, self.sem).start(priority=prio)

    def wait(self):
        pltpu.make_async_copy(self.whole, self.whole, self.sem).wait()


def _kernel(x_hbm, k_hbm, v_hbm, wq_hbm, wo_hbm, wg_hbm, wu_hbm, wd_hbm, c_hbm, wm_hbm,
            o_ref,
            x_v, c_v, wm_v, wq_v, wo_v, wg_v, wu_v, wd_v, kbuf, vbuf, q_v, sems,
            *, W, look, wrow0, ppc):
    B, H, S, Dh = k_hbm.shape
    D = x_v.shape[-1]
    F = wd_v.shape[0]
    nsem = sems.shape[0]
    nch, _, ck, _ = kbuf.shape
    nb = B // 2

    counter = [0]

    def next_sem():
        i = counter[0] % nsem
        counter[0] += 1
        return sems.at[i]

    def weight_pieces(src, dst, rows, ncol):
        g, r, cdim = src.shape
        cw = cdim // ncol
        out = []
        for i in range(r // rows):
            for cc in range(ncol):
                for g0 in range(0, g, 4):
                    idx = (pl.ds(g0, 4), pl.ds(i * rows, rows), pl.ds(cc * cw, cw))
                    out.append(_Piece(src.at[idx], dst.at[idx], 1, next_sem()))
        return out

    pro = [_Piece(c_hbm, c_v, B, next_sem()), _Piece(x_hbm, x_v, B, next_sem())]
    pro += weight_pieces(wm_hbm, wm_v, 8, 2)
    n_mod = len(pro)
    pro += weight_pieces(wq_hbm, wq_v, 8, 2)
    n_q = len(pro)
    pro += weight_pieces(wo_hbm, wo_v, 32, 1)

    n_head = 2 * nch * (B // nb)
    assert nsem == n_head and look + ppc <= n_head
    sem0 = counter[0]

    def head_pieces(h):
        out = []
        for src, dst in ((k_hbm, kbuf), (v_hbm, vbuf)):
            for c in range(nch):
                for b0 in range(0, B, nb):
                    out.append(_Piece(src.at[pl.ds(b0, nb), h, pl.ds(S - W + c * ck, ck)],
                                      dst.at[c, pl.ds(b0, nb)], 1,
                                      sems.at[(sem0 + len(out)) % nsem]))
        return out

    fchunks = [(f, min(128, F - f)) for f in range(0, F, 128)]
    epi = []
    for f, n in fchunks:
        for src, dst in ((wg_hbm, wg_v), (wu_hbm, wu_v), (wd_hbm, wd_v)):
            epi.append(_Piece(src.at[pl.ds(f, n)], dst.at[pl.ds(f, n)], wrow0, next_sem()))

    def advance(cur, nxt, j):
        cur[j].wait()
        t = j + look
        if t < len(cur):
            cur[t].start()
        elif t - len(cur) < len(nxt):
            nxt[t - len(cur)].start()

    head0 = head_pieces(0)
    for p in pro[:look]:
        p.start()
    for j in range(n_mod):
        advance(pro, head0, j)
    c = c_v[...].astype(_F32)
    sc = (c * jax.nn.sigmoid(c)).astype(_BF16)
    mod = jnp.dot(sc, wm_v[...].reshape(D, 6 * D), preferred_element_type=_F32)
    sa, ca, ga, sb, cb, gb = [mod[:, i * D:(i + 1) * D] for i in range(6)]
    x = x_v[...].astype(_F32)
    h1 = (_layernorm(x) * (1.0 + ca) + sa).astype(_BF16)
    for j in range(n_mod, n_q):
        advance(pro, head0, j)
    q = jnp.dot(h1, wq_v[...].reshape(D, H * Dh), preferred_element_type=_F32) * (Dh ** -0.5)
    for h in range(H):
        q_v[h] = q[:, h * Dh:(h + 1) * Dh]
    for j in range(n_q, len(pro)):
        advance(pro, head0, j)

    row = jax.lax.broadcasted_iota(jnp.int32, (B, ck), 0)
    cpg = ppc * nb // B
    hpg = H // _G

    def head(h, nxt, a_out):
        cur = head_pieces(h)
        qh = q_v[h].astype(_BF16)
        nk = n_head // 2
        s = []
        for c0 in range(0, nch, cpg):
            for j in range(ppc):
                advance(cur, nxt, c0 * (B // nb) + j)
            for c in range(c0, c0 + cpg):
                sp = jax.lax.dot_general(qh, kbuf[c].reshape(B * ck, Dh), _NT,
                                         preferred_element_type=_F32)
                sc_ = sp[:, :ck]
                for b in range(1, B):
                    sc_ = jnp.where(row == b, sp[:, b * ck:(b + 1) * ck], sc_)
                s.append(sc_)
        m = jnp.max(functools.reduce(jnp.maximum, s), axis=-1, keepdims=True)
        p = [jnp.exp(t - m) for t in s]
        l = jnp.sum(functools.reduce(jnp.add, p), axis=-1, keepdims=True)
        o = jnp.zeros((B, Dh), _F32)
        for c0 in range(0, nch, cpg):
            for j in range(ppc):
                advance(cur, nxt, nk + c0 * (B // nb) + j)
            for c in range(c0, c0 + cpg):
                pd = jnp.concatenate([jnp.where(row == b, p[c], 0.0) for b in range(B)],
                                     axis=-1).astype(_BF16)
                o = o + jnp.dot(pd, vbuf[c].reshape(B * ck, Dh), preferred_element_type=_F32)
        att = (o / l).astype(_BF16)
        ro = (h % hpg) * Dh
        if not isinstance(h, int):
            ro = pl.multiple_of(ro, Dh)
        return a_out + jnp.dot(att, wo_v[h // hpg, pl.ds(ro, Dh), :], preferred_element_type=_F32)

    a_out = jax.lax.fori_loop(0, H - 1, lambda h, acc: head(h, head_pieces(h + 1), acc),
                              jnp.zeros((B, D), _F32))
    a_out = head(H - 1, epi, a_out)

    x1 = x + ga * a_out
    h2 = (_layernorm(x1) * (1.0 + cb) + sb).astype(_BF16)
    acc = jnp.zeros((B, D), _F32)
    for i, (f, n) in enumerate(fchunks):
        advance(epi, [], 3 * i)
        g = jax.lax.dot_general(h2, wg_v[pl.ds(f, n), :], _NT, preferred_element_type=_F32)
        advance(epi, [], 3 * i + 1)
        u = jax.lax.dot_general(h2, wu_v[pl.ds(f, n), :], _NT, preferred_element_type=_F32)
        hh = (jax.nn.sigmoid(g) * u).astype(_BF16)
        advance(epi, [], 3 * i + 2)
        acc = acc + jnp.dot(hh, wd_v[pl.ds(f, n), :], preferred_element_type=_F32)
    o_ref[...] = (x1 + gb * acc).astype(o_ref.dtype)


def _forward(A_x, A_k_cache, A_v_cache, A_wq, A_wo, B_w_gate, B_w_up, B_w_down, c, w_mod,
             look=12, wrow0=32, ppc=2, nobounds=True):
    B, Sq, D = A_x.shape
    _, H, S, Dh = A_k_cache.shape
    F = B_w_down.shape[0]
    W = min(4096, max(256, S // 4))
    ck = 128
    nsem = 2 * (W // ck) * 2
    slab = lambda w: w.reshape(_G, w.shape[0] // _G, w.shape[1])
    wm, wq, wo = slab(w_mod), slab(A_wq), slab(A_wo)
    any_spec = pl.BlockSpec(memory_space=pl.ANY)
    out = pl.pallas_call(
        functools.partial(_kernel, W=W, look=look, wrow0=wrow0, ppc=ppc),
        in_specs=[any_spec] * 10,
        out_specs=pl.BlockSpec(memory_space=pltpu.VMEM),
        out_shape=jax.ShapeDtypeStruct((B, D), A_x.dtype),
        scratch_shapes=[
            pltpu.VMEM((B, D), _BF16),
            pltpu.VMEM((B, D), _BF16),
            pltpu.VMEM(wm.shape, _BF16),
            pltpu.VMEM(wq.shape, _BF16),
            pltpu.VMEM(wo.shape, _BF16),
            pltpu.VMEM((F, D), _BF16),
            pltpu.VMEM((F, D), _BF16),
            pltpu.VMEM((F, D), _BF16),
            pltpu.VMEM((W // ck, B, ck, Dh), _BF16),
            pltpu.VMEM((W // ck, B, ck, Dh), _BF16),
            pltpu.VMEM((H, B, Dh), _F32),
            pltpu.SemaphoreType.DMA((nsem,)),
        ],
        compiler_params=pltpu.CompilerParams(vmem_limit_bytes=64 * 1024 * 1024,
                                             disable_bounds_checks=nobounds),
    )(A_x.reshape(B, D), A_k_cache, A_v_cache, wq, wo, B_w_gate.T, B_w_up.T, B_w_down, c, wm)
    return out.reshape(B, Sq, D)


@jax.jit
def pallas_adaLN_cond__sliding_block_cached__glu_gated_glu__decode_kernel(
    A_x: jax.Array,
    A_k_cache: jax.Array,
    A_v_cache: jax.Array,
    A_wq: jax.Array,
    A_wo: jax.Array,
    B_x: jax.Array,
    B_w_gate: jax.Array,
    B_w_up: jax.Array,
    B_w_down: jax.Array,
    c: jax.Array,
    w_mod: jax.Array,
):
    del B_x
    return _forward(A_x, A_k_cache, A_v_cache, A_wq, A_wo, B_w_gate, B_w_up, B_w_down, c, w_mod)
```

```python
import functools

import jax
import jax.numpy as jnp
import jax.experimental.pallas as pl
import jax.experimental.pallas.tpu as pltpu

_NT = (((1,), (1,)), ((), ()))
_EPS = 1e-5
_F32 = jnp.float32
_BF16 = jnp.bfloat16
_G = 8


def _layernorm(x):
    m = jnp.mean(x, axis=-1, keepdims=True)
    xc = x - m
    v = jnp.mean(xc * xc, axis=-1, keepdims=True)
    return xc * jax.lax.rsqrt(v + _EPS)


class _Piece:
    def __init__(self, src, dst, n0, sem):
        n = dst.shape[0]
        n0 = min(n0, n)
        self.parts = []
        if n0 > 0:
            self.parts.append((src.at[pl.ds(0, n0)], dst.at[pl.ds(0, n0)], 0))
        if n0 < n:
            self.parts.append((src.at[pl.ds(n0, n - n0)], dst.at[pl.ds(n0, n - n0)], 1))
        self.whole, self.sem = dst, sem

    def start(self, priority):
        for src, dst, prio in self.parts:
            if prio == priority:
                pltpu.make_async_copy(src, dst, self.sem).start(priority=prio)

    def wait(self):
        pltpu.make_async_copy(self.whole, self.whole, self.sem).wait()


def _kernel(x_hbm, k_hbm, v_hbm, wq_hbm, wo_hbm, wg_hbm, wu_hbm, wd_hbm, c_hbm, wm_hbm,
            o_ref,
            x_v, c_v, wm_v, wq_v, wo_v, wg_v, wu_v, wd_v, kbuf, vbuf, q_v, sems,
            *, W, look, look0, wrow0, ppc):
    B, H, S, Dh = k_hbm.shape
    D = x_v.shape[-1]
    F = wd_v.shape[0]
    nsem = sems.shape[0]
    nch, _, ck, _ = kbuf.shape
    nb = B // 2

    counter = [0]

    def next_sem():
        i = counter[0] % nsem
        counter[0] += 1
        return sems.at[i]

    def weight_pieces(src, dst, rows, ncol):
        g, r, cdim = src.shape
        cw = cdim // ncol
        out = []
        for i in range(r // rows):
            for cc in range(ncol):
                for g0 in range(0, g, 4):
                    idx = (pl.ds(g0, 4), pl.ds(i * rows, rows), pl.ds(cc * cw, cw))
                    out.append(_Piece(src.at[idx], dst.at[idx], 1, next_sem()))
        return out

    pro = [_Piece(c_hbm, c_v, B, next_sem()), _Piece(x_hbm, x_v, B, next_sem())]
    pro += weight_pieces(wm_hbm, wm_v, 8, 2)
    n_mod = len(pro)
    pro += weight_pieces(wq_hbm, wq_v, 8, 2)
    n_q = len(pro)
    pro += weight_pieces(wo_hbm, wo_v, 32, 1)

    n_head = 2 * nch * (B // nb)
    assert nsem == n_head and max(look, look0) + ppc <= n_head
    sem0 = counter[0]

    def head_pieces(h):
        out = []
        for src, dst in ((k_hbm, kbuf), (v_hbm, vbuf)):
            for c in range(nch):
                for b0 in range(0, B, nb):
                    out.append(_Piece(src.at[pl.ds(b0, nb), h, pl.ds(S - W + c * ck, ck)],
                                      dst.at[c, pl.ds(b0, nb)], 1,
                                      sems.at[(sem0 + len(out)) % nsem]))
        return out

    fchunks = [(f, min(128, F - f)) for f in range(0, F, 128)]
    epi = []
    for f, n in fchunks:
        for src, dst in ((wg_hbm, wg_v), (wu_hbm, wu_v), (wd_hbm, wd_v)):
            epi.append(_Piece(src.at[pl.ds(f, n)], dst.at[pl.ds(f, n)], wrow0, next_sem()))

    def advance(cur, nxt, j):
        cur[j].wait()
        for prio, ahead in ((0, look0), (1, look)):
            t = j + ahead
            if t < len(cur):
                cur[t].start(prio)
            elif t - len(cur) < len(nxt):
                nxt[t - len(cur)].start(prio)

    head0 = head_pieces(0)
    for j in range(max(look, look0)):
        if j < look0:
            pro[j].start(0)
        if j < look:
            pro[j].start(1)
    for j in range(n_mod):
        advance(pro, head0, j)
    c = c_v[...].astype(_F32)
    sc = (c * jax.nn.sigmoid(c)).astype(_BF16)
    mod = jnp.dot(sc, wm_v[...].reshape(D, 6 * D), preferred_element_type=_F32)
    sa, ca, ga, sb, cb, gb = [mod[:, i * D:(i + 1) * D] for i in range(6)]
    x = x_v[...].astype(_F32)
    h1 = (_layernorm(x) * (1.0 + ca) + sa).astype(_BF16)
    for j in range(n_mod, n_q):
        advance(pro, head0, j)
    q = jnp.dot(h1, wq_v[...].reshape(D, H * Dh), preferred_element_type=_F32) * (Dh ** -0.5)
    for h in range(H):
        q_v[h] = q[:, h * Dh:(h + 1) * Dh]
    for j in range(n_q, len(pro)):
        advance(pro, head0, j)

    row = jax.lax.broadcasted_iota(jnp.int32, (B, ck), 0)
    cpg = ppc * nb // B
    hpg = H // _G

    def head(h, nxt, a_out):
        cur = head_pieces(h)
        qh = q_v[h].astype(_BF16)
        nk = n_head // 2
        s = []
        for c0 in range(0, nch, cpg):
            for j in range(ppc):
                advance(cur, nxt, c0 * (B // nb) + j)
            for c in range(c0, c0 + cpg):
                sp = jax.lax.dot_general(qh, kbuf[c].reshape(B * ck, Dh), _NT,
                                         preferred_element_type=_F32)
                sc_ = sp[:, :ck]
                for b in range(1, B):
                    sc_ = jnp.where(row == b, sp[:, b * ck:(b + 1) * ck], sc_)
                s.append(sc_)
        m = jnp.max(functools.reduce(jnp.maximum, s), axis=-1, keepdims=True)
        p = [jnp.exp(t - m) for t in s]
        l = jnp.sum(functools.reduce(jnp.add, p), axis=-1, keepdims=True)
        o = jnp.zeros((B, Dh), _F32)
        for c0 in range(0, nch, cpg):
            for j in range(ppc):
                advance(cur, nxt, nk + c0 * (B // nb) + j)
            for c in range(c0, c0 + cpg):
                pd = jnp.concatenate([jnp.where(row == b, p[c], 0.0) for b in range(B)],
                                     axis=-1).astype(_BF16)
                o = o + jnp.dot(pd, vbuf[c].reshape(B * ck, Dh), preferred_element_type=_F32)
        att = (o / l).astype(_BF16)
        ro = (h % hpg) * Dh
        if not isinstance(h, int):
            ro = pl.multiple_of(ro, Dh)
        return a_out + jnp.dot(att, wo_v[h // hpg, pl.ds(ro, Dh), :], preferred_element_type=_F32)

    a_out = jax.lax.fori_loop(0, H - 1, lambda h, acc: head(h, head_pieces(h + 1), acc),
                              jnp.zeros((B, D), _F32))
    a_out = head(H - 1, epi, a_out)

    x1 = x + ga * a_out
    h2 = (_layernorm(x1) * (1.0 + cb) + sb).astype(_BF16)
    acc = jnp.zeros((B, D), _F32)
    for i, (f, n) in enumerate(fchunks):
        advance(epi, [], 3 * i)
        g = jax.lax.dot_general(h2, wg_v[pl.ds(f, n), :], _NT, preferred_element_type=_F32)
        advance(epi, [], 3 * i + 1)
        u = jax.lax.dot_general(h2, wu_v[pl.ds(f, n), :], _NT, preferred_element_type=_F32)
        hh = (jax.nn.sigmoid(g) * u).astype(_BF16)
        advance(epi, [], 3 * i + 2)
        acc = acc + jnp.dot(hh, wd_v[pl.ds(f, n), :], preferred_element_type=_F32)
    o_ref[...] = (x1 + gb * acc).astype(o_ref.dtype)


def _forward(A_x, A_k_cache, A_v_cache, A_wq, A_wo, B_w_gate, B_w_up, B_w_down, c, w_mod,
             look=16, look0=20, wrow0=32, ppc=2, nobounds=True):
    B, Sq, D = A_x.shape
    _, H, S, Dh = A_k_cache.shape
    F = B_w_down.shape[0]
    W = min(4096, max(256, S // 4))
    ck = 128
    nsem = 2 * (W // ck) * 2
    slab = lambda w: w.reshape(_G, w.shape[0] // _G, w.shape[1])
    wm, wq, wo = slab(w_mod), slab(A_wq), slab(A_wo)
    any_spec = pl.BlockSpec(memory_space=pl.ANY)
    out = pl.pallas_call(
        functools.partial(_kernel, W=W, look=look, look0=look0, wrow0=wrow0, ppc=ppc),
        in_specs=[any_spec] * 10,
        out_specs=pl.BlockSpec(memory_space=pltpu.VMEM),
        out_shape=jax.ShapeDtypeStruct((B, D), A_x.dtype),
        scratch_shapes=[
            pltpu.VMEM((B, D), _BF16),
            pltpu.VMEM((B, D), _BF16),
            pltpu.VMEM(wm.shape, _BF16),
            pltpu.VMEM(wq.shape, _BF16),
            pltpu.VMEM(wo.shape, _BF16),
            pltpu.VMEM((F, D), _BF16),
            pltpu.VMEM((F, D), _BF16),
            pltpu.VMEM((F, D), _BF16),
            pltpu.VMEM((W // ck, B, ck, Dh), _BF16),
            pltpu.VMEM((W // ck, B, ck, Dh), _BF16),
            pltpu.VMEM((H, B, Dh), _F32),
            pltpu.SemaphoreType.DMA((nsem,)),
        ],
        compiler_params=pltpu.CompilerParams(vmem_limit_bytes=64 * 1024 * 1024,
                                             disable_bounds_checks=nobounds,
                                             disable_semaphore_checks=nobounds),
    )(A_x.reshape(B, D), A_k_cache, A_v_cache, wq, wo, B_w_gate.T, B_w_up.T, B_w_down, c, wm)
    return out.reshape(B, Sq, D)


@jax.jit
def pallas_adaLN_cond__sliding_block_cached__glu_gated_glu__decode_kernel(
    A_x: jax.Array,
    A_k_cache: jax.Array,
    A_v_cache: jax.Array,
    A_wq: jax.Array,
    A_wo: jax.Array,
    B_x: jax.Array,
    B_w_gate: jax.Array,
    B_w_up: jax.Array,
    B_w_down: jax.Array,
    c: jax.Array,
    w_mod: jax.Array,
):
    del B_x
    return _forward(A_x, A_k_cache, A_v_cache, A_wq, A_wo, B_w_gate, B_w_up, B_w_down, c, w_mod)
```

```python
import functools

import jax
import jax.numpy as jnp
import jax.experimental.pallas as pl
import jax.experimental.pallas.tpu as pltpu

_NT = (((1,), (1,)), ((), ()))
_EPS = 1e-5
_F32 = jnp.float32
_BF16 = jnp.bfloat16
_G = 8
_R = 8
_CK = 128


def _layernorm(x):
    m = jnp.mean(x, axis=-1, keepdims=True)
    xc = x - m
    v = jnp.mean(xc * xc, axis=-1, keepdims=True)
    return xc * jax.lax.rsqrt(v + _EPS)


class _Piece:
    def __init__(self, src, dst, n0, sem):
        n = dst.shape[0]
        n0 = min(n0, n)
        self.parts = []
        if n0 > 0:
            self.parts.append((src.at[pl.ds(0, n0)], dst.at[pl.ds(0, n0)], 0))
        if n0 < n:
            self.parts.append((src.at[pl.ds(n0, n - n0)], dst.at[pl.ds(n0, n - n0)], 1))
        self.whole, self.sem = dst, sem

    def start(self, priority):
        for src, dst, prio in self.parts:
            if prio == priority:
                pltpu.make_async_copy(src, dst, self.sem).start(priority=prio)

    def wait(self):
        pltpu.make_async_copy(self.whole, self.whole, self.sem).wait()


class _Stream:
    def __init__(self, cur, nxt, looks):
        self.cur, self.all, self.looks, self.pos = cur, cur + nxt, looks, 0

    def advance(self, n=1):
        for _ in range(n):
            self.cur[self.pos].wait()
            for prio, ahead in enumerate(self.looks):
                if self.pos + ahead < len(self.all):
                    self.all[self.pos + ahead].start(prio)
            self.pos += 1

    def advance_to(self, pos):
        self.advance(pos - self.pos)


def _kernel(x_hbm, k_hbm, v_hbm, wq_hbm, wo_hbm, wg_hbm, wu_hbm, wd_hbm, c_hbm, wm_hbm,
            o_ref,
            x_v, c_v, wm_v, wq_v, wo_v, wg_v, wu_v, wd_v, kbuf, vbuf, mod_v, q_v, att_v, sems,
            *, W, looks, wrow0, dlag):
    B, D = x_v.shape
    _, nu, H2, S, Dh = k_hbm.shape
    H = 2 * H2
    F = wd_v.shape[0]
    nsem = sems.shape[0]
    nch = W // _CK
    n_steps = B * H // _R

    counter = [0]

    def next_sem():
        i = counter[0] % nsem
        counter[0] += 1
        return sems.at[i]

    def weight_pieces(src, dst, rows, ncol):
        g, r, cdim = src.shape
        cw = cdim // ncol
        out = []
        for i in range(r // rows):
            for cc in range(ncol):
                for g0 in range(0, g, 4):
                    idx = (pl.ds(g0, 4), pl.ds(i * rows, rows), pl.ds(cc * cw, cw))
                    out.append(_Piece(src.at[idx], dst.at[idx], 1, next_sem()))
        return out

    pro = [_Piece(c_hbm, c_v, B, next_sem()), _Piece(x_hbm, x_v, B, next_sem())]
    pro += weight_pieces(wm_hbm, wm_v, 8, 2)
    n_mod = len(pro)
    pro += weight_pieces(wq_hbm, wq_v, 8, 2)
    n_q = len(pro)
    pro += weight_pieces(wo_hbm, wo_v, 32, 1)

    ppc = _R // nu
    assert nsem == 2 * nch * ppc and max(looks) + ppc <= nsem
    sem0 = counter[0]

    def step_pieces(i):
        out = []
        for src, dst in ((k_hbm, kbuf), (v_hbm, vbuf)):
            for c in range(nch):
                for g in range(ppc):
                    out.append(_Piece(
                        src.at[(i % 2) * ppc + g, :, i // 2, pl.ds(S - W + c * _CK, _CK)],
                        dst.at[c, pl.ds(g * nu, nu)], 1, sems.at[(sem0 + len(out)) % nsem]))
        return out

    fchunks = [(f, min(128, F - f)) for f in range(0, F, 128)]
    nf = len(fchunks)
    epi = []
    for i in range(nf + dlag):
        todo = []
        if i < nf:
            todo += [(wg_hbm, wg_v, i), (wu_hbm, wu_v, i)]
        if i >= dlag:
            todo += [(wd_hbm, wd_v, i - dlag)]
        for src, dst, t in todo:
            sl = pl.ds(*fchunks[t])
            epi.append(_Piece(src.at[sl], dst.at[sl], wrow0, next_sem()))

    st = _Stream(pro, step_pieces(0), looks)
    for j in range(max(looks)):
        for prio, ahead in enumerate(looks):
            if j < ahead:
                pro[j].start(prio)
    att_v[...] = jnp.zeros(att_v.shape, _F32)
    st.advance(2)
    c = c_v[...].astype(_F32)
    sc = (c * jax.nn.sigmoid(c)).astype(_BF16)
    xn = _layernorm(x_v[...].astype(_F32))
    st.advance_to(n_mod)
    for t in range(6):
        w = wm_v[:, :, t * D:(t + 1) * D].reshape(D, D)
        mod_v[t] = jnp.dot(sc, w, preferred_element_type=_F32)
        st.advance(2)
    h1 = (xn * (1.0 + mod_v[1]) + mod_v[0]).astype(_BF16)
    st.advance_to(n_q)
    hq = 4
    for h0 in range(0, H, hq):
        w = wq_v[:, :, h0 * Dh:(h0 + hq) * Dh].reshape(D, hq * Dh)
        q = jnp.dot(h1, w, preferred_element_type=_F32) * (Dh ** -0.5)
        for h in range(h0, h0 + hq):
            q_v[pl.ds((h % H2) * 2 * _R + h // H2, B, stride=2), :] = (
                q[:, (h - h0) * Dh:(h - h0 + 1) * Dh])
        st.advance(2)
    st.advance_to(len(pro))

    row = jax.lax.broadcasted_iota(jnp.int32, (_R, _CK), 0)
    hpg = H // _G

    def project(t, a_out):
        h = t // 2 + (t % 2) * H2
        att = att_v[pl.ds((t // 2) * 2 * _R + t % 2, B, stride=2), :].astype(_BF16)
        ro = (h % hpg) * Dh
        if not isinstance(t, int):
            ro = pl.multiple_of(ro, Dh)
        return a_out + jnp.dot(att, wo_v[h // hpg, pl.ds(ro, Dh), :], preferred_element_type=_F32)

    def step(i, nxt, a_out):
        st = _Stream(step_pieces(i), nxt, looks)
        r0 = i * _R if isinstance(i, int) else pl.multiple_of(i * _R, _R)
        qs = q_v[pl.ds(r0, _R), :].astype(_BF16)
        s = []
        for c in range(nch):
            st.advance(ppc)
            sp = jax.lax.dot_general(qs, kbuf[c].reshape(_R * _CK, Dh), _NT,
                                     preferred_element_type=_F32)
            sd = sp[:, :_CK]
            for r in range(1, _R):
                sd = jnp.where(row == r, sp[:, r * _CK:(r + 1) * _CK], sd)
            s.append(sd)
            if c == 0:
                a_out = project((i + n_steps - 2) % n_steps, a_out)
        st.advance(1)
        m = jnp.max(functools.reduce(jnp.maximum, s), axis=-1, keepdims=True)
        p = [jnp.exp(t - m) for t in s]
        l = jnp.sum(functools.reduce(jnp.add, p), axis=-1, keepdims=True)
        o = jnp.zeros((_R, Dh), _F32)
        for c in range(nch):
            st.advance_to((nch + c + 1) * ppc)
            pd = jnp.concatenate([jnp.where(row == r, p[c], 0.0) for r in range(_R)],
                                 axis=-1).astype(_BF16)
            o = o + jnp.dot(pd, vbuf[c].reshape(_R * _CK, Dh), preferred_element_type=_F32)
        att_v[pl.ds(r0, _R), :] = o / l
        return a_out

    a_out = jax.lax.fori_loop(0, n_steps - 1, lambda i, acc: step(i, step_pieces(i + 1), acc),
                              jnp.zeros((B, D), _F32))
    a_out = step(n_steps - 1, epi, a_out)

    st = _Stream(epi, [], looks)
    st.advance(1)
    a_out = project(n_steps - 1, project(n_steps - 2, a_out))
    x1 = x_v[...].astype(_F32) + mod_v[2] * a_out
    st.advance(1)
    h2 = (_layernorm(x1) * (1.0 + mod_v[4]) + mod_v[3]).astype(_BF16)
    acc = jnp.zeros((B, D), _F32)
    hh = []
    pos = 0
    for i in range(nf + dlag):
        pos += (2 if i < nf else 0) + (1 if i >= dlag else 0)
        st.advance_to(pos)
        if i < nf:
            sl = pl.ds(*fchunks[i])
            g = jax.lax.dot_general(h2, wg_v[sl, :], _NT, preferred_element_type=_F32)
            u = jax.lax.dot_general(h2, wu_v[sl, :], _NT, preferred_element_type=_F32)
            hh.append((jax.nn.sigmoid(g) * u).astype(_BF16))
        if i >= dlag:
            sl = pl.ds(*fchunks[i - dlag])
            acc = acc + jnp.dot(hh[i - dlag], wd_v[sl, :], preferred_element_type=_F32)
    o_ref[...] = (x1 + mod_v[5] * acc).astype(o_ref.dtype)


def _forward(A_x, A_k_cache, A_v_cache, A_wq, A_wo, B_w_gate, B_w_up, B_w_down, c, w_mod,
             look=16, look0=16, wrow0=32, dlag=2, nochecks=True):
    B, Sq, D = A_x.shape
    _, H, S, Dh = A_k_cache.shape
    F = B_w_down.shape[0]
    W = min(4096, max(256, S // 4))
    nch = W // _CK
    slab = lambda w: w.reshape(_G, w.shape[0] // _G, w.shape[1])
    wm, wq, wo = slab(w_mod), slab(A_wq), slab(A_wo)
    kv_shape = (B // 2, 4, H // 2, S, Dh)
    any_spec = pl.BlockSpec(memory_space=pl.ANY)
    out = pl.pallas_call(
        functools.partial(_kernel, W=W, looks=(look0, look), wrow0=wrow0, dlag=dlag),
        in_specs=[any_spec] * 10,
        out_specs=pl.BlockSpec(memory_space=pltpu.VMEM),
        out_shape=jax.ShapeDtypeStruct((B, D), A_x.dtype),
        scratch_shapes=[
            pltpu.VMEM((B, D), _BF16),
            pltpu.VMEM((B, D), _BF16),
            pltpu.VMEM(wm.shape, _BF16),
            pltpu.VMEM(wq.shape, _BF16),
            pltpu.VMEM(wo.shape, _BF16),
            pltpu.VMEM((F, D), _BF16),
            pltpu.VMEM((F, D), _BF16),
            pltpu.VMEM((F, D), _BF16),
            pltpu.VMEM((nch, _R, _CK, Dh), _BF16),
            pltpu.VMEM((nch, _R, _CK, Dh), _BF16),
            pltpu.VMEM((6, B, D), _F32),
            pltpu.VMEM((B * H, Dh), _F32),
            pltpu.VMEM((B * H, Dh), _F32),
            pltpu.SemaphoreType.DMA((4 * nch,)),
        ],
        compiler_params=pltpu.CompilerParams(vmem_limit_bytes=64 * 1024 * 1024,
                                             disable_bounds_checks=nochecks,
                                             disable_semaphore_checks=nochecks),
    )(A_x.reshape(B, D), A_k_cache.reshape(kv_shape), A_v_cache.reshape(kv_shape), wq, wo,
      B_w_gate.T, B_w_up.T, B_w_down, c, wm)
    return out.reshape(B, Sq, D)


@jax.jit
def pallas_adaLN_cond__sliding_block_cached__glu_gated_glu__decode_kernel(
    A_x: jax.Array,
    A_k_cache: jax.Array,
    A_v_cache: jax.Array,
    A_wq: jax.Array,
    A_wo: jax.Array,
    B_x: jax.Array,
    B_w_gate: jax.Array,
    B_w_up: jax.Array,
    B_w_down: jax.Array,
    c: jax.Array,
    w_mod: jax.Array,
):
    del B_x
    return _forward(A_x, A_k_cache, A_v_cache, A_wq, A_wo, B_w_gate, B_w_up, B_w_down, c, w_mod)
```

```python
import functools

import jax
import jax.numpy as jnp
import jax.experimental.pallas as pl
import jax.experimental.pallas.tpu as pltpu

_NT = (((1,), (1,)), ((), ()))
_EPS = 1e-5
_F32 = jnp.float32
_BF16 = jnp.bfloat16
_R = 8
_CK = 128
_FC = 32


def _layernorm(x):
    m = jnp.mean(x, axis=-1, keepdims=True)
    xc = x - m
    v = jnp.mean(xc * xc, axis=-1, keepdims=True)
    return xc * jax.lax.rsqrt(v + _EPS)


class _Piece:
    def __init__(self, parts, sem, whole=None):
        self.parts, self.sem, self.whole = parts, sem, whole

    def start(self):
        for src, dst, prio in self.parts:
            pltpu.make_async_copy(src, dst, self.sem).start(priority=prio)

    def wait(self):
        if self.whole is not None:
            pltpu.make_async_copy(self.whole, self.whole, self.sem).wait()
        else:
            for src, dst, _ in self.parts:
                pltpu.make_async_copy(src, dst, self.sem).wait()


def _split_piece(src, dst, sem):
    n = dst.shape[0]
    return _Piece([(src.at[pl.ds(0, 1)], dst.at[pl.ds(0, 1)], 0),
                   (src.at[pl.ds(1, n - 1)], dst.at[pl.ds(1, n - 1)], 1)], sem, dst)


class _Stream:
    def __init__(self, cur, nxt, look):
        self.cur, self.all, self.look, self.pos = cur, cur + nxt, look, 0

    def advance(self, n=1):
        for _ in range(n):
            self.cur[self.pos].wait()
            if self.pos + self.look < len(self.all):
                self.all[self.pos + self.look].start()
            self.pos += 1

    def advance_to(self, pos):
        self.advance(pos - self.pos)


def _kernel(x_hbm, k_hbm, v_hbm, wq_hbm, wo_hbm, wg_hbm, wu_hbm, wd_hbm, c_hbm, wm_hbm,
            o_ref,
            x_v, c_v, wm_v, wq_v, wo_v, wg_v, wu_v, wd_v, kbuf, vbuf, mod_v, q_v, att_v, sems,
            *, W, look, dlag):
    B, D = x_v.shape
    _, nu, H2, S, Dh = k_hbm.shape
    H = 2 * H2
    F = wd_v.shape[0]
    nsem = sems.shape[0]
    nch = W // _CK
    n_steps = B * H // _R

    counter = [0]

    def next_sem():
        i = counter[0] % nsem
        counter[0] += 1
        return sems.at[i]

    def weight_blocks(src, dst, rows, ncol):
        _, g, r, cdim = src.shape
        cw = cdim // ncol
        idxs = [(slice(None), gi, pl.ds(i * rows, rows), pl.ds(cc * cw, cw))
                for i in range(r // rows) for cc in range(ncol) for gi in range(g)]
        return [(src.at[idx], dst.at[idx]) for idx in idxs]

    pro = [_Piece([(c_hbm, c_v, 0)], next_sem()), _Piece([(x_hbm, x_v, 0)], next_sem())]
    for pair in zip(weight_blocks(wm_hbm, wm_v, 8, 2), weight_blocks(wq_hbm, wq_v, 8, 2),
                    strict=True):
        pro += [_split_piece(src, dst, next_sem()) for src, dst in pair]
    n_mq = len(pro)
    pro += [_split_piece(src, dst, next_sem())
            for src, dst in weight_blocks(wo_hbm, wo_v, 32, 1)]

    ppc = _R // nu
    assert nsem == 2 * nch * ppc and look + ppc <= nsem
    sem0 = counter[0]

    def step_pieces(i):
        out = []
        for src, dst in ((k_hbm, kbuf), (v_hbm, vbuf)):
            for c in range(nch):
                for g in range(ppc):
                    out.append(_split_piece(
                        src.at[(i % 2) * ppc + g, :, i // 2, pl.ds(S - W + c * _CK, _CK)],
                        dst.at[c, pl.ds(g * nu, nu)], sems.at[(sem0 + len(out)) % nsem]))
        return out

    nfc = F // _FC
    half = (nfc + 1) // 2
    perm = [(s % 2) * half + s // 2 for s in range(nfc)]
    spt = 128 // _FC
    first = nfc % spt
    bounds = ([0] if first else []) + list(range(first, nfc + 1, spt))
    tiles = list(zip(bounds[:-1], bounds[1:]))
    seq = []
    for s in range(nfc + dlag):
        if s < nfc:
            seq += [(0, s), (1, s)]
        if s >= dlag:
            seq += [(2, s - dlag)]
    groups = [seq[max(e - 4, 0):e] for e in range(len(seq), 0, -4)][::-1]
    epi, ready = [], {}
    ffn_refs = ((wg_hbm, wg_v), (wu_hbm, wu_v), (wd_hbm, wd_v))
    for j, grp in enumerate(groups):
        parts = []
        for t, (a, s) in enumerate(grp):
            src, dst = ffn_refs[a]
            prio = 0 if t == 0 and j < len(groups) - 1 else 1
            parts.append((src.at[pl.ds(perm[s] * _FC, _FC)], dst.at[pl.ds(s * _FC, _FC)], prio))
            ready[(a, s)] = j + 1
        epi.append(_Piece(parts, next_sem()))

    st = _Stream(pro, step_pieces(0), look)
    for p in pro[:look]:
        p.start()
    att_v[...] = jnp.zeros(att_v.shape, _F32)
    st.advance(2)
    c = c_v[...].astype(_F32)
    sc = (c * jax.nn.sigmoid(c)).astype(_BF16)
    xn = _layernorm(x_v[...].astype(_F32))
    st.advance_to(n_mq)
    for t in range(6):
        w = wm_v[:, :, :, t * D:(t + 1) * D].reshape(D, D)
        mod_v[t] = jnp.dot(sc, w, preferred_element_type=_F32)
        st.advance(2)
    h1 = (xn * (1.0 + mod_v[1]) + mod_v[0]).astype(_BF16)
    hq = 4
    for h0 in range(0, H, hq):
        w = wq_v[:, :, :, h0 * Dh:(h0 + hq) * Dh].reshape(D, hq * Dh)
        q = jnp.dot(h1, w, preferred_element_type=_F32) * (Dh ** -0.5)
        for h in range(h0, h0 + hq):
            q_v[pl.ds((h % H2) * 2 * _R + h // H2, B, stride=2), :] = (
                q[:, (h - h0) * Dh:(h - h0 + 1) * Dh])
        st.advance(2)
    st.advance_to(len(pro))

    row = jax.lax.broadcasted_iota(jnp.int32, (_R, _CK), 0)
    hps = wo_v.shape[2] // Dh

    def project(t, a_out):
        h = t // 2 + (t % 2) * H2
        att = att_v[pl.ds((t // 2) * 2 * _R + t % 2, B, stride=2), :].astype(_BF16)
        ro = (h % hps) * Dh
        if not isinstance(t, int):
            ro = pl.multiple_of(ro, Dh)
        w = wo_v[h // (2 * hps), (h // hps) % 2, pl.ds(ro, Dh), :]
        return a_out + jnp.dot(att, w, preferred_element_type=_F32)

    def step(i, nxt, a_out):
        st = _Stream(step_pieces(i), nxt, look)
        r0 = i * _R if isinstance(i, int) else pl.multiple_of(i * _R, _R)
        qs = q_v[pl.ds(r0, _R), :].astype(_BF16)
        s = []
        for c in range(nch):
            st.advance(ppc)
            sp = jax.lax.dot_general(qs, kbuf[c].reshape(_R * _CK, Dh), _NT,
                                     preferred_element_type=_F32)
            sd = sp[:, :_CK]
            for r in range(1, _R):
                sd = jnp.where(row == r, sp[:, r * _CK:(r + 1) * _CK], sd)
            s.append(sd)
            if c == 0:
                a_out = project((i + n_steps - 2) % n_steps, a_out)
        st.advance(1)
        m = jnp.max(functools.reduce(jnp.maximum, s), axis=-1, keepdims=True)
        p = [jnp.exp(t - m) for t in s]
        l = jnp.sum(functools.reduce(jnp.add, p), axis=-1, keepdims=True)
        o = jnp.zeros((_R, Dh), _F32)
        for c in range(nch):
            st.advance_to((nch + c + 1) * ppc)
            pd = jnp.concatenate([jnp.where(row == r, p[c], 0.0) for r in range(_R)],
                                 axis=-1).astype(_BF16)
            o = o + jnp.dot(pd, vbuf[c].reshape(_R * _CK, Dh), preferred_element_type=_F32)
        att_v[pl.ds(r0, _R), :] = o / l
        return a_out

    a_out = jax.lax.fori_loop(0, n_steps - 1, lambda i, acc: step(i, step_pieces(i + 1), acc),
                              jnp.zeros((B, D), _F32))
    a_out = step(n_steps - 1, epi, a_out)

    st = _Stream(epi, [], look)
    st.advance(1)
    a_out = project(n_steps - 1, project(n_steps - 2, a_out))
    x1 = x_v[...].astype(_F32) + mod_v[2] * a_out
    st.advance(1)
    h2 = (_layernorm(x1) * (1.0 + mod_v[4]) + mod_v[3]).astype(_BF16)
    acc = jnp.zeros((B, D), _F32)
    hh = []
    nd = 0
    while nd < len(tiles):
        if len(hh) < len(tiles):
            pos = ready[(1, tiles[len(hh)][1] - 1)]
        else:
            pos = ready[(2, tiles[nd][1] - 1)]
        st.advance_to(max(pos, st.pos))
        have = len(hh)
        if have < len(tiles):
            lo, hi = tiles[have]
            sl = pl.ds(lo * _FC, (hi - lo) * _FC)
            g = jax.lax.dot_general(h2, wg_v[sl, :], _NT, preferred_element_type=_F32)
            u = jax.lax.dot_general(h2, wu_v[sl, :], _NT, preferred_element_type=_F32)
            hh.append((jax.nn.sigmoid(g) * u).astype(_BF16))
        while nd < have and ready[(2, tiles[nd][1] - 1)] <= st.pos:
            lo, hi = tiles[nd]
            acc = acc + jnp.dot(hh[nd], wd_v[pl.ds(lo * _FC, (hi - lo) * _FC), :],
                                preferred_element_type=_F32)
            nd += 1
    assert st.pos == len(epi)
    o_ref[...] = (x1 + mod_v[5] * acc).astype(o_ref.dtype)


def _forward(A_x, A_k_cache, A_v_cache, A_wq, A_wo, B_w_gate, B_w_up, B_w_down, c, w_mod,
             look=10, dlag=8, nochecks=True):
    B, Sq, D = A_x.shape
    _, H, S, Dh = A_k_cache.shape
    F = B_w_down.shape[0]
    W = min(4096, max(256, S // 4))
    nch = W // _CK
    slab = lambda w: w.reshape(4, 2, w.shape[0] // 8, w.shape[1])
    wm, wq, wo = slab(w_mod), slab(A_wq), slab(A_wo)
    kv_shape = (B // 2, 4, H // 2, S, Dh)
    any_spec = pl.BlockSpec(memory_space=pl.ANY)
    out = pl.pallas_call(
        functools.partial(_kernel, W=W, look=look, dlag=dlag),
        in_specs=[any_spec] * 10,
        out_specs=pl.BlockSpec(memory_space=pltpu.VMEM),
        out_shape=jax.ShapeDtypeStruct((B, D), A_x.dtype),
        scratch_shapes=[
            pltpu.VMEM((B, D), _BF16),
            pltpu.VMEM((B, D), _BF16),
            pltpu.VMEM(wm.shape, _BF16),
            pltpu.VMEM(wq.shape, _BF16),
            pltpu.VMEM(wo.shape, _BF16),
            pltpu.VMEM((F, D), _BF16),
            pltpu.VMEM((F, D), _BF16),
            pltpu.VMEM((F, D), _BF16),
            pltpu.VMEM((nch, _R, _CK, Dh), _BF16),
            pltpu.VMEM((nch, _R, _CK, Dh), _BF16),
            pltpu.VMEM((6, B, D), _F32),
            pltpu.VMEM((B * H + _R, Dh), _F32),
            pltpu.VMEM((B * H + _R, Dh), _F32),
            pltpu.SemaphoreType.DMA((4 * nch,)),
        ],
        compiler_params=pltpu.CompilerParams(vmem_limit_bytes=64 * 1024 * 1024,
                                             disable_bounds_checks=nochecks,
                                             disable_semaphore_checks=nochecks),
    )(A_x.reshape(B, D), A_k_cache.reshape(kv_shape), A_v_cache.reshape(kv_shape), wq, wo,
      B_w_gate.T, B_w_up.T, B_w_down, c, wm)
    return out.reshape(B, Sq, D)


@jax.jit
def pallas_adaLN_cond__sliding_block_cached__glu_gated_glu__decode_kernel(
    A_x: jax.Array,
    A_k_cache: jax.Array,
    A_v_cache: jax.Array,
    A_wq: jax.Array,
    A_wo: jax.Array,
    B_x: jax.Array,
    B_w_gate: jax.Array,
    B_w_up: jax.Array,
    B_w_down: jax.Array,
    c: jax.Array,
    w_mod: jax.Array,
):
    del B_x
    return _forward(A_x, A_k_cache, A_v_cache, A_wq, A_wo, B_w_gate, B_w_up, B_w_down, c, w_mod)
```

```python
import functools

import jax
import jax.numpy as jnp
import jax.experimental.pallas as pl
import jax.experimental.pallas.tpu as pltpu

_NT = (((1,), (1,)), ((), ()))
_EPS = 1e-5
_F32 = jnp.float32
_BF16 = jnp.bfloat16
_R = 8
_CK = 128
_FC = 32


def _layernorm(x):
    m = jnp.mean(x, axis=-1, keepdims=True)
    xc = x - m
    v = jnp.mean(xc * xc, axis=-1, keepdims=True)
    return xc * jax.lax.rsqrt(v + _EPS)


class _Piece:
    def __init__(self, parts, sem, whole=None):
        self.parts, self.sem, self.whole = parts, sem, whole

    def start(self):
        for src, dst, prio in self.parts:
            pltpu.make_async_copy(src, dst, self.sem).start(priority=prio)

    def wait(self):
        if self.whole is not None:
            pltpu.make_async_copy(self.whole, self.whole, self.sem).wait()
        else:
            for src, dst, _ in self.parts:
                pltpu.make_async_copy(src, dst, self.sem).wait()


def _split(src, dst):
    n = dst.shape[0]
    return [(src.at[pl.ds(0, 1)], dst.at[pl.ds(0, 1)], 0),
            (src.at[pl.ds(1, n - 1)], dst.at[pl.ds(1, n - 1)], 1)]


def _split_piece(src, dst, sem):
    return _Piece(_split(src, dst), sem, dst)


class _Stream:
    def __init__(self, cur, nxt, look):
        self.cur, self.all, self.look, self.pos = cur, cur + nxt, look, 0

    def advance(self, n=1):
        for _ in range(n):
            self.cur[self.pos].wait()
            if self.pos + self.look < len(self.all):
                self.all[self.pos + self.look].start()
            self.pos += 1

    def advance_to(self, pos):
        self.advance(pos - self.pos)


def _kernel(x_hbm, k_hbm, v_hbm, wq_hbm, wo_hbm, wg_hbm, wu_hbm, wd_hbm, c_hbm, wm_hbm,
            o_ref,
            x_v, c_v, wm_v, wq_v, wo_v, wg_v, wu_v, wd_v, kbuf, vbuf, mod_v, q_v, att_v, sems,
            *, W, look, dlag, shift):
    B, D = x_v.shape
    _, nu, H2, S, Dh = k_hbm.shape
    H = 2 * H2
    F = wd_v.shape[0]
    nsem = sems.shape[0]
    nch = W // _CK
    n_steps = B * H // _R

    counter = [0]

    def next_sem():
        i = counter[0] % nsem
        counter[0] += 1
        return sems.at[i]

    def weight_blocks(src, dst, rows, ncol):
        _, g, r, cdim = src.shape
        cw = cdim // ncol
        idxs = [(slice(None), gi, pl.ds(i * rows, rows), pl.ds(cc * cw, cw))
                for i in range(r // rows) for cc in range(ncol) for gi in range(g)]
        return [(src.at[idx], dst.at[idx]) for idx in idxs]

    pro = [_Piece([(c_hbm, c_v, 0)], next_sem()), _Piece([(x_hbm, x_v, 0)], next_sem())]
    for pair in zip(weight_blocks(wm_hbm, wm_v, 8, 2), weight_blocks(wq_hbm, wq_v, 8, 2),
                    strict=True):
        pro += [_split_piece(src, dst, next_sem()) for src, dst in pair]
    n_mq = len(pro)
    pro += [_split_piece(src, dst, next_sem())
            for src, dst in weight_blocks(wo_hbm, wo_v, 32, 1)]

    ppc = _R // nu
    assert nsem == 2 * nch * ppc and look + ppc <= nsem
    sem0 = counter[0]

    spans = [[((c - 1) * _CK + shift, _CK, 0)] for c in range(nch)]
    spans[0] = [(W - _CK + shift, _CK - shift, 0)] + ([(0, shift, _CK - shift)] if shift else [])

    def step_pieces(i):
        out = []
        for src, dst in ((k_hbm, kbuf), (v_hbm, vbuf)):
            for c in range(nch):
                for g in range(ppc):
                    blk = dst.at[c, pl.ds(g * nu, nu)]
                    parts = []
                    for lo, n, off in spans[c]:
                        parts += _split(
                            src.at[(i % 2) * ppc + g, :, i // 2, pl.ds(S - W + lo, n)],
                            blk.at[:, pl.ds(off, n)])
                    out.append(_Piece(parts, sems.at[(sem0 + len(out)) % nsem], blk))
        return out

    nfc = F // _FC
    half = (nfc + 1) // 2
    perm = [(s % 2) * half + s // 2 for s in range(nfc)]
    spt = 128 // _FC
    first = nfc % spt
    bounds = ([0] if first else []) + list(range(first, nfc + 1, spt))
    tiles = list(zip(bounds[:-1], bounds[1:]))
    seq = []
    for s in range(nfc + dlag):
        if s < nfc:
            seq += [(0, s), (1, s)]
        if s >= dlag:
            seq += [(2, s - dlag)]
    groups = [seq[max(e - 4, 0):e] for e in range(len(seq), 0, -4)][::-1]
    epi, ready = [], {}
    ffn_refs = ((wg_hbm, wg_v), (wu_hbm, wu_v), (wd_hbm, wd_v))
    for j, grp in enumerate(groups):
        parts = []
        for t, (a, s) in enumerate(grp):
            src, dst = ffn_refs[a]
            prio = 0 if t == 0 and j < len(groups) - 1 else 1
            parts.append((src.at[pl.ds(perm[s] * _FC, _FC)], dst.at[pl.ds(s * _FC, _FC)], prio))
            ready[(a, s)] = j + 1
        epi.append(_Piece(parts, next_sem()))

    st = _Stream(pro, step_pieces(0), look)
    for p in pro[:look]:
        p.start()
    att_v[...] = jnp.zeros(att_v.shape, _F32)
    st.advance(2)
    c = c_v[...].astype(_F32)
    sc = (c * jax.nn.sigmoid(c)).astype(_BF16)
    xn = _layernorm(x_v[...].astype(_F32))
    st.advance_to(n_mq)
    for t in range(6):
        w = wm_v[:, :, :, t * D:(t + 1) * D].reshape(D, D)
        mod_v[t] = jnp.dot(sc, w, preferred_element_type=_F32)
        st.advance(2)
    h1 = (xn * (1.0 + mod_v[1]) + mod_v[0]).astype(_BF16)
    hq = 4
    for h0 in range(0, H, hq):
        w = wq_v[:, :, :, h0 * Dh:(h0 + hq) * Dh].reshape(D, hq * Dh)
        q = jnp.dot(h1, w, preferred_element_type=_F32) * (Dh ** -0.5)
        for h in range(h0, h0 + hq):
            q_v[pl.ds((h % H2) * 2 * _R + h // H2, B, stride=2), :] = (
                q[:, (h - h0) * Dh:(h - h0 + 1) * Dh])
        st.advance(2)
    st.advance_to(len(pro))

    row = jax.lax.broadcasted_iota(jnp.int32, (_R, _CK), 0)
    hps = wo_v.shape[2] // Dh

    def project(t, a_out):
        h = t // 2 + (t % 2) * H2
        att = att_v[pl.ds((t // 2) * 2 * _R + t % 2, B, stride=2), :].astype(_BF16)
        ro = (h % hps) * Dh
        if not isinstance(t, int):
            ro = pl.multiple_of(ro, Dh)
        w = wo_v[h // (2 * hps), (h // hps) % 2, pl.ds(ro, Dh), :]
        return a_out + jnp.dot(att, w, preferred_element_type=_F32)

    def step(i, nxt, a_out):
        st = _Stream(step_pieces(i), nxt, look)
        r0 = i * _R if isinstance(i, int) else pl.multiple_of(i * _R, _R)
        qs = q_v[pl.ds(r0, _R), :].astype(_BF16)
        s = []
        for c in range(nch):
            st.advance(ppc)
            sp = jax.lax.dot_general(qs, kbuf[c].reshape(_R * _CK, Dh), _NT,
                                     preferred_element_type=_F32)
            sd = sp[:, :_CK]
            for r in range(1, _R):
                sd = jnp.where(row == r, sp[:, r * _CK:(r + 1) * _CK], sd)
            s.append(sd)
            if c == 0:
                a_out = project((i + n_steps - 2) % n_steps, a_out)
        st.advance(1)
        m = jnp.max(functools.reduce(jnp.maximum, s), axis=-1, keepdims=True)
        p = [jnp.exp(t - m) for t in s]
        l = jnp.sum(functools.reduce(jnp.add, p), axis=-1, keepdims=True)
        o = jnp.zeros((_R, Dh), _F32)
        for c in range(nch):
            st.advance_to((nch + c + 1) * ppc)
            pd = jnp.concatenate([jnp.where(row == r, p[c], 0.0) for r in range(_R)],
                                 axis=-1).astype(_BF16)
            o = o + jnp.dot(pd, vbuf[c].reshape(_R * _CK, Dh), preferred_element_type=_F32)
        att_v[pl.ds(r0, _R), :] = o / l
        return a_out

    a_out = jax.lax.fori_loop(0, n_steps - 1, lambda i, acc: step(i, step_pieces(i + 1), acc),
                              jnp.zeros((B, D), _F32))
    a_out = step(n_steps - 1, epi, a_out)

    st = _Stream(epi, [], look)
    st.advance(1)
    a_out = project(n_steps - 1, project(n_steps - 2, a_out))
    x1 = x_v[...].astype(_F32) + mod_v[2] * a_out
    st.advance(1)
    h2 = (_layernorm(x1) * (1.0 + mod_v[4]) + mod_v[3]).astype(_BF16)
    acc = jnp.zeros((B, D), _F32)
    hh = []
    nd = 0
    while nd < len(tiles):
        if len(hh) < len(tiles):
            pos = ready[(1, tiles[len(hh)][1] - 1)]
        else:
            pos = ready[(2, tiles[nd][1] - 1)]
        st.advance_to(max(pos, st.pos))
        have = len(hh)
        if have < len(tiles):
            lo, hi = tiles[have]
            sl = pl.ds(lo * _FC, (hi - lo) * _FC)
            g = jax.lax.dot_general(h2, wg_v[sl, :], _NT, preferred_element_type=_F32)
            u = jax.lax.dot_general(h2, wu_v[sl, :], _NT, preferred_element_type=_F32)
            hh.append((jax.nn.sigmoid(g) * u).astype(_BF16))
        while nd < have and ready[(2, tiles[nd][1] - 1)] <= st.pos:
            lo, hi = tiles[nd]
            acc = acc + jnp.dot(hh[nd], wd_v[pl.ds(lo * _FC, (hi - lo) * _FC), :],
                                preferred_element_type=_F32)
            nd += 1
    assert st.pos == len(epi)
    o_ref[...] = (x1 + mod_v[5] * acc).astype(o_ref.dtype)


def _forward(A_x, A_k_cache, A_v_cache, A_wq, A_wo, B_w_gate, B_w_up, B_w_down, c, w_mod,
             look=10, dlag=8, shift=8, nochecks=True):
    B, Sq, D = A_x.shape
    _, H, S, Dh = A_k_cache.shape
    F = B_w_down.shape[0]
    W = min(4096, max(256, S // 4))
    nch = W // _CK
    slab = lambda w: w.reshape(4, 2, w.shape[0] // 8, w.shape[1])
    wm, wq, wo = slab(w_mod), slab(A_wq), slab(A_wo)
    kv_shape = (B // 2, 4, H // 2, S, Dh)
    any_spec = pl.BlockSpec(memory_space=pl.ANY)
    out = pl.pallas_call(
        functools.partial(_kernel, W=W, look=look, dlag=dlag, shift=shift),
        in_specs=[any_spec] * 10,
        out_specs=pl.BlockSpec(memory_space=pltpu.VMEM),
        out_shape=jax.ShapeDtypeStruct((B, D), A_x.dtype),
        scratch_shapes=[
            pltpu.VMEM((B, D), _BF16),
            pltpu.VMEM((B, D), _BF16),
            pltpu.VMEM(wm.shape, _BF16),
            pltpu.VMEM(wq.shape, _BF16),
            pltpu.VMEM(wo.shape, _BF16),
            pltpu.VMEM((F, D), _BF16),
            pltpu.VMEM((F, D), _BF16),
            pltpu.VMEM((F, D), _BF16),
            pltpu.VMEM((nch, _R, _CK, Dh), _BF16),
            pltpu.VMEM((nch, _R, _CK, Dh), _BF16),
            pltpu.VMEM((6, B, D), _F32),
            pltpu.VMEM((B * H + _R, Dh), _F32),
            pltpu.VMEM((B * H + _R, Dh), _F32),
            pltpu.SemaphoreType.DMA((4 * nch,)),
        ],
        compiler_params=pltpu.CompilerParams(vmem_limit_bytes=64 * 1024 * 1024,
                                             disable_bounds_checks=nochecks,
                                             disable_semaphore_checks=nochecks),
    )(A_x.reshape(B, D), A_k_cache.reshape(kv_shape), A_v_cache.reshape(kv_shape), wq, wo,
      B_w_gate.T, B_w_up.T, B_w_down, c, wm)
    return out.reshape(B, Sq, D)


@jax.jit
def pallas_adaLN_cond__sliding_block_cached__glu_gated_glu__decode_kernel(
    A_x: jax.Array,
    A_k_cache: jax.Array,
    A_v_cache: jax.Array,
    A_wq: jax.Array,
    A_wo: jax.Array,
    B_x: jax.Array,
    B_w_gate: jax.Array,
    B_w_up: jax.Array,
    B_w_down: jax.Array,
    c: jax.Array,
    w_mod: jax.Array,
):
    del B_x
    return _forward(A_x, A_k_cache, A_v_cache, A_wq, A_wo, B_w_gate, B_w_up, B_w_down, c, w_mod)
```

```python
import functools

import jax
import jax.numpy as jnp
import jax.experimental.pallas as pl
import jax.experimental.pallas.tpu as pltpu

_NT = (((1,), (1,)), ((), ()))
_EPS = 1e-5
_F32 = jnp.float32
_BF16 = jnp.bfloat16
_R = 8
_CK = 128
_FC = 32


def _layernorm(x):
    m = jnp.mean(x, axis=-1, keepdims=True)
    xc = x - m
    v = jnp.mean(xc * xc, axis=-1, keepdims=True)
    return xc * jax.lax.rsqrt(v + _EPS)


class _Piece:
    def __init__(self, parts, sem, whole=None):
        self.parts, self.sem, self.whole = parts, sem, whole

    def start(self):
        for src, dst, prio in self.parts:
            pltpu.make_async_copy(src, dst, self.sem).start(priority=prio)

    def wait(self):
        if self.whole is not None:
            pltpu.make_async_copy(self.whole, self.whole, self.sem).wait()
        else:
            for src, dst, _ in self.parts:
                pltpu.make_async_copy(src, dst, self.sem).wait()


def _split(src, dst):
    n = dst.shape[0]
    return [(src.at[pl.ds(0, 1)], dst.at[pl.ds(0, 1)], 0),
            (src.at[pl.ds(1, n - 1)], dst.at[pl.ds(1, n - 1)], 1)]


def _split_piece(src, dst, sem):
    return _Piece(_split(src, dst), sem, dst)


class _Stream:
    def __init__(self, cur, nxt, look):
        self.cur, self.all, self.look, self.pos = cur, cur + nxt, look, 0

    def advance(self, n=1):
        for _ in range(n):
            self.cur[self.pos].wait()
            if self.pos + self.look < len(self.all):
                self.all[self.pos + self.look].start()
            self.pos += 1

    def advance_to(self, pos):
        self.advance(pos - self.pos)


def _kernel(x_hbm, k_hbm, v_hbm, wq_hbm, wo_hbm, wg_hbm, wu_hbm, wd_hbm, c_hbm, wm_hbm,
            o_ref,
            x_v, c_v, wm_v, wq_v, wo_v, wg_v, wu_v, wd_v, kbuf, vbuf, mod_v, q_v, att_v, sems,
            *, W, look, dlag, shift):
    B, D = x_v.shape
    _, _, H2, S, Dh = k_hbm.shape
    H = 2 * H2
    F = wd_v.shape[0]
    nsem = sems.shape[0]
    nch = W // _CK
    n_steps = B * H // _R

    counter = [0]

    def next_sem():
        i = counter[0] % nsem
        counter[0] += 1
        return sems.at[i]

    def weight_blocks(src, dst, rows, ncol):
        _, g, r, cdim = src.shape
        cw = cdim // ncol
        idxs = [(slice(None), gi, pl.ds(i * rows, rows), pl.ds(cc * cw, cw))
                for i in range(r // rows) for cc in range(ncol) for gi in range(g)]
        return [(src.at[idx], dst.at[idx]) for idx in idxs]

    pro = [_Piece([(c_hbm, c_v, 0)], next_sem()), _Piece([(x_hbm, x_v, 0)], next_sem())]
    for pair in zip(weight_blocks(wm_hbm, wm_v, 8, 2), weight_blocks(wq_hbm, wq_v, 8, 2),
                    strict=True):
        pro += [_split_piece(src, dst, next_sem()) for src, dst in pair]
    n_mq = len(pro)
    pro += [_split_piece(src, dst, next_sem())
            for src, dst in weight_blocks(wo_hbm, wo_v, 32, 1)]

    ppc = 2
    n1 = _R // ppc - 1
    assert nsem == 2 * nch * ppc and look + ppc <= nsem
    sem0 = counter[0]

    spans = [[((c - 1) * _CK + shift, _CK, 0)] for c in range(nch)]
    spans[0] = [(W - _CK + shift, _CK - shift, 0)] + ([(0, shift, _CK - shift)] if shift else [])

    def step_pieces(i):
        out = []
        for src, dst in ((k_hbm, kbuf), (v_hbm, vbuf)):
            for c in range(nch):
                for g in range(ppc):
                    parts = [(src.at[i % 2, us, i // 2, pl.ds(S - W + lo, n)],
                              dst.at[c, us, pl.ds(off, n)], prio)
                             for lo, n, off in spans[c]
                             for prio, us in enumerate((pl.ds(g, 1), pl.ds(ppc + g * n1, n1)))]
                    out.append(_Piece(parts, sems.at[(sem0 + len(out)) % nsem]))
        return out

    nfc = F // _FC
    half = (nfc + 1) // 2
    perm = [(s % 2) * half + s // 2 for s in range(nfc)]
    spt = 128 // _FC
    first = nfc % spt
    bounds = ([0] if first else []) + list(range(first, nfc + 1, spt))
    tiles = list(zip(bounds[:-1], bounds[1:]))
    seq = []
    for s in range(nfc + dlag):
        if s < nfc:
            seq += [(0, s), (1, s)]
        if s >= dlag:
            seq += [(2, s - dlag)]
    groups = [seq[max(e - 4, 0):e] for e in range(len(seq), 0, -4)][::-1]
    epi, ready = [], {}
    ffn_refs = ((wg_hbm, wg_v), (wu_hbm, wu_v), (wd_hbm, wd_v))
    for j, grp in enumerate(groups):
        parts = []
        for t, (a, s) in enumerate(grp):
            src, dst = ffn_refs[a]
            prio = 0 if t == 0 and j < len(groups) - 1 else 1
            parts.append((src.at[pl.ds(perm[s] * _FC, _FC)], dst.at[pl.ds(s * _FC, _FC)], prio))
            ready[(a, s)] = j + 1
        epi.append(_Piece(parts, next_sem()))

    st = _Stream(pro, step_pieces(0), look)
    for p in pro[:look]:
        p.start()
    att_v[...] = jnp.zeros(att_v.shape, _F32)
    st.advance(2)
    c = c_v[...].astype(_F32)
    sc = (c * jax.nn.sigmoid(c)).astype(_BF16)
    xn = _layernorm(x_v[...].astype(_F32))
    st.advance_to(n_mq)
    for t in range(6):
        w = wm_v[:, :, :, t * D:(t + 1) * D].reshape(D, D)
        mod_v[t] = jnp.dot(sc, w, preferred_element_type=_F32)
        st.advance(2)
    h1 = (xn * (1.0 + mod_v[1]) + mod_v[0]).astype(_BF16)
    hq = 4
    for h0 in range(0, H, hq):
        w = wq_v[:, :, :, h0 * Dh:(h0 + hq) * Dh].reshape(D, hq * Dh)
        q = jnp.dot(h1, w, preferred_element_type=_F32) * (Dh ** -0.5)
        for h in range(h0, h0 + hq):
            q_v[pl.ds((h % H2) * 2 * _R + h // H2, B, stride=2), :] = (
                q[:, (h - h0) * Dh:(h - h0 + 1) * Dh])
        st.advance(2)
    st.advance_to(len(pro))

    row = jax.lax.broadcasted_iota(jnp.int32, (_R, _CK), 0)
    hps = wo_v.shape[2] // Dh

    def project(t, a_out):
        h = t // 2 + (t % 2) * H2
        att = att_v[pl.ds((t // 2) * 2 * _R + t % 2, B, stride=2), :].astype(_BF16)
        ro = (h % hps) * Dh
        if not isinstance(t, int):
            ro = pl.multiple_of(ro, Dh)
        w = wo_v[h // (2 * hps), (h // hps) % 2, pl.ds(ro, Dh), :]
        return a_out + jnp.dot(att, w, preferred_element_type=_F32)

    def step(i, nxt, a_out):
        st = _Stream(step_pieces(i), nxt, look)
        r0 = i * _R if isinstance(i, int) else pl.multiple_of(i * _R, _R)
        qs = q_v[pl.ds(r0, _R), :].astype(_BF16)
        s = []
        for c in range(nch):
            st.advance(ppc)
            sp = jax.lax.dot_general(qs, kbuf[c].reshape(_R * _CK, Dh), _NT,
                                     preferred_element_type=_F32)
            sd = sp[:, :_CK]
            for r in range(1, _R):
                sd = jnp.where(row == r, sp[:, r * _CK:(r + 1) * _CK], sd)
            s.append(sd)
            if c == 0:
                a_out = project((i + n_steps - 2) % n_steps, a_out)
        st.advance(1)
        m = jnp.max(functools.reduce(jnp.maximum, s), axis=-1, keepdims=True)
        p = [jnp.exp(t - m) for t in s]
        l = jnp.sum(functools.reduce(jnp.add, p), axis=-1, keepdims=True)
        o = jnp.zeros((_R, Dh), _F32)
        for c in range(nch):
            st.advance_to((nch + c + 1) * ppc)
            pd = jnp.concatenate([jnp.where(row == r, p[c], 0.0) for r in range(_R)],
                                 axis=-1).astype(_BF16)
            o = o + jnp.dot(pd, vbuf[c].reshape(_R * _CK, Dh), preferred_element_type=_F32)
        att_v[pl.ds(r0, _R), :] = o / l
        return a_out

    a_out = jax.lax.fori_loop(0, n_steps - 1, lambda i, acc: step(i, step_pieces(i + 1), acc),
                              jnp.zeros((B, D), _F32))
    a_out = step(n_steps - 1, epi, a_out)

    st = _Stream(epi, [], look)
    st.advance(1)
    a_out = project(n_steps - 1, project(n_steps - 2, a_out))
    x1 = x_v[...].astype(_F32) + mod_v[2] * a_out
    st.advance(1)
    h2 = (_layernorm(x1) * (1.0 + mod_v[4]) + mod_v[3]).astype(_BF16)
    acc = jnp.zeros((B, D), _F32)
    hh = []
    nd = 0
    while nd < len(tiles):
        if len(hh) < len(tiles):
            pos = ready[(1, tiles[len(hh)][1] - 1)]
        else:
            pos = ready[(2, tiles[nd][1] - 1)]
        st.advance_to(max(pos, st.pos))
        have = len(hh)
        if have < len(tiles):
            lo, hi = tiles[have]
            sl = pl.ds(lo * _FC, (hi - lo) * _FC)
            g = jax.lax.dot_general(h2, wg_v[sl, :], _NT, preferred_element_type=_F32)
            u = jax.lax.dot_general(h2, wu_v[sl, :], _NT, preferred_element_type=_F32)
            hh.append((jax.nn.sigmoid(g) * u).astype(_BF16))
        while nd < have and ready[(2, tiles[nd][1] - 1)] <= st.pos:
            lo, hi = tiles[nd]
            acc = acc + jnp.dot(hh[nd], wd_v[pl.ds(lo * _FC, (hi - lo) * _FC), :],
                                preferred_element_type=_F32)
            nd += 1
    assert st.pos == len(epi)
    o_ref[...] = (x1 + mod_v[5] * acc).astype(o_ref.dtype)


def _forward(A_x, A_k_cache, A_v_cache, A_wq, A_wo, B_w_gate, B_w_up, B_w_down, c, w_mod,
             look=10, dlag=8, shift=8, nochecks=True):
    B, Sq, D = A_x.shape
    _, H, S, Dh = A_k_cache.shape
    F = B_w_down.shape[0]
    W = min(4096, max(256, S // 4))
    nch = W // _CK
    slab = lambda w: w.reshape(4, 2, w.shape[0] // 8, w.shape[1])
    wm, wq, wo = slab(w_mod), slab(A_wq), slab(A_wo)
    kv_shape = (B // 4, _R, H // 2, S, Dh)
    any_spec = pl.BlockSpec(memory_space=pl.ANY)
    out = pl.pallas_call(
        functools.partial(_kernel, W=W, look=look, dlag=dlag, shift=shift),
        in_specs=[any_spec] * 10,
        out_specs=pl.BlockSpec(memory_space=pltpu.VMEM),
        out_shape=jax.ShapeDtypeStruct((B, D), A_x.dtype),
        scratch_shapes=[
            pltpu.VMEM((B, D), _BF16),
            pltpu.VMEM((B, D), _BF16),
            pltpu.VMEM(wm.shape, _BF16),
            pltpu.VMEM(wq.shape, _BF16),
            pltpu.VMEM(wo.shape, _BF16),
            pltpu.VMEM((F, D), _BF16),
            pltpu.VMEM((F, D), _BF16),
            pltpu.VMEM((F, D), _BF16),
            pltpu.VMEM((nch, _R, _CK, Dh), _BF16),
            pltpu.VMEM((nch, _R, _CK, Dh), _BF16),
            pltpu.VMEM((6, B, D), _F32),
            pltpu.VMEM((B * H + _R, Dh), _F32),
            pltpu.VMEM((B * H + _R, Dh), _F32),
            pltpu.SemaphoreType.DMA((4 * nch,)),
        ],
        compiler_params=pltpu.CompilerParams(vmem_limit_bytes=64 * 1024 * 1024,
                                             disable_bounds_checks=nochecks,
                                             disable_semaphore_checks=nochecks),
    )(A_x.reshape(B, D), A_k_cache.reshape(kv_shape), A_v_cache.reshape(kv_shape), wq, wo,
      B_w_gate.T, B_w_up.T, B_w_down, c, wm)
    return out.reshape(B, Sq, D)


@jax.jit
def pallas_adaLN_cond__sliding_block_cached__glu_gated_glu__decode_kernel(
    A_x: jax.Array,
    A_k_cache: jax.Array,
    A_v_cache: jax.Array,
    A_wq: jax.Array,
    A_wo: jax.Array,
    B_x: jax.Array,
    B_w_gate: jax.Array,
    B_w_up: jax.Array,
    B_w_down: jax.Array,
    c: jax.Array,
    w_mod: jax.Array,
):
    del B_x
    return _forward(A_x, A_k_cache, A_v_cache, A_wq, A_wo, B_w_gate, B_w_up, B_w_down, c, w_mod)
```

```python
import functools

import jax
import jax.numpy as jnp
import jax.experimental.pallas as pl
import jax.experimental.pallas.tpu as pltpu

_NT = (((1,), (1,)), ((), ()))
_EPS = 1e-5
_F32 = jnp.float32
_BF16 = jnp.bfloat16
_CK = 128
_FC = 32


def _layernorm(x):
    m = jnp.mean(x, axis=-1, keepdims=True)
    xc = x - m
    v = jnp.mean(xc * xc, axis=-1, keepdims=True)
    return xc * jax.lax.rsqrt(v + _EPS)


class _Piece:
    def __init__(self, parts, sem, whole=None):
        self.parts, self.sem, self.whole = parts, sem, whole

    def start(self):
        for src, dst, prio in self.parts:
            pltpu.make_async_copy(src, dst, self.sem).start(priority=prio)

    def wait(self):
        if self.whole is not None:
            pltpu.make_async_copy(self.whole, self.whole, self.sem).wait()
        else:
            for src, dst, _ in self.parts:
                pltpu.make_async_copy(src, dst, self.sem).wait()


def _split(src, dst):
    n = dst.shape[0]
    return [(src.at[pl.ds(0, 1)], dst.at[pl.ds(0, 1)], 0),
            (src.at[pl.ds(1, n - 1)], dst.at[pl.ds(1, n - 1)], 1)]


def _split_piece(src, dst, sem):
    return _Piece(_split(src, dst), sem, dst)


class _Stream:
    def __init__(self, cur, nxt, look):
        self.cur, self.all, self.look, self.pos = cur, cur + nxt, look, 0

    def advance(self, n=1):
        for _ in range(n):
            self.cur[self.pos].wait()
            if self.pos + self.look < len(self.all):
                self.all[self.pos + self.look].start()
            self.pos += 1

    def advance_to(self, pos):
        self.advance(pos - self.pos)


def _kernel(x_hbm, k_hbm, v_hbm, wq_hbm, wo_hbm, wg_hbm, wu_hbm, wd_hbm, c_hbm, wm_hbm,
            o_ref,
            x_v, c_v, wm_v, wq_v, wo_v, wg_v, wu_v, wd_v, kbuf, vbuf, mod_v, q_v, att_v, sems,
            *, W, look, dlag, shift, runs, koffs, voffs):
    B, D = x_v.shape
    nu, H2, S, Dh = k_hbm.shape
    H = 2 * H2
    F = wd_v.shape[0]
    nsem = sems.shape[0]
    nch = W // _CK
    n_steps = H2

    counter = [0]

    def next_sem():
        i = counter[0] % nsem
        counter[0] += 1
        return sems.at[i]

    def weight_blocks(src, dst, rows, ncol):
        _, g, r, cdim = src.shape
        cw = cdim // ncol
        idxs = [(slice(None), gi, pl.ds(i * rows, rows), pl.ds(cc * cw, cw))
                for i in range(r // rows) for cc in range(ncol) for gi in range(g)]
        return [(src.at[idx], dst.at[idx]) for idx in idxs]

    pro = [_Piece([(c_hbm, c_v, 0)], next_sem()), _Piece([(x_hbm, x_v, 0)], next_sem())]
    for pair in zip(weight_blocks(wm_hbm, wm_v, 8, 2), weight_blocks(wq_hbm, wq_v, 8, 2),
                    strict=True):
        pro += [_split_piece(src, dst, next_sem()) for src, dst in pair]
    n_mq = len(pro)
    pro += [_split_piece(src, dst, next_sem())
            for src, dst in weight_blocks(wo_hbm, wo_v, 32, 1)]

    ppc = len(runs)
    assert ppc + sum(runs) == nu
    starts = [ppc + sum(runs[:g]) for g in range(ppc)]
    assert (2 * nch * ppc) % nsem == 0 and look < nsem
    sem0 = counter[0]

    spans = [[((c - 1) * _CK + shift, _CK, 0)] for c in range(nch)]
    spans[0] = [(W - _CK + shift, _CK - shift, 0)] + ([(0, shift, _CK - shift)] if shift else [])

    def step_pieces(i):
        out = []
        for src, dst in ((k_hbm, kbuf), (v_hbm, vbuf)):
            for c in range(nch):
                for g in range(ppc):
                    parts = [(src.at[us, i, pl.ds(S - W + lo, n)],
                              dst.at[c, us, pl.ds(off, n)], prio)
                             for lo, n, off in spans[c]
                             for prio, us in enumerate((pl.ds(g, 1), pl.ds(starts[g], runs[g])))]
                    out.append(_Piece(parts, sems.at[(sem0 + len(out)) % nsem]))
        return out

    nfc = F // _FC
    half = (nfc + 1) // 2
    perm = [(s % 2) * half + s // 2 for s in range(nfc)]
    spt = 128 // _FC
    first = nfc % spt
    bounds = ([0] if first else []) + list(range(first, nfc + 1, spt))
    tiles = list(zip(bounds[:-1], bounds[1:]))
    seq = []
    for s in range(nfc + dlag):
        if s < nfc:
            seq += [(0, s), (1, s)]
        if s >= dlag:
            seq += [(2, s - dlag)]
    groups = [seq[max(e - 4, 0):e] for e in range(len(seq), 0, -4)][::-1]
    epi, ready = [], {}
    ffn_refs = ((wg_hbm, wg_v), (wu_hbm, wu_v), (wd_hbm, wd_v))
    for j, grp in enumerate(groups):
        parts = []
        for t, (a, s) in enumerate(grp):
            src, dst = ffn_refs[a]
            prio = 0 if t == 0 and j < len(groups) - 1 else 1
            parts.append((src.at[pl.ds(perm[s] * _FC, _FC)], dst.at[pl.ds(s * _FC, _FC)], prio))
            ready[(a, s)] = j + 1
        epi.append(_Piece(parts, next_sem()))

    st = _Stream(pro, step_pieces(0), look)
    for p in pro[:look]:
        p.start()
    att_v[...] = jnp.zeros(att_v.shape, _F32)
    st.advance(2)
    c = c_v[...].astype(_F32)
    sc = (c * jax.nn.sigmoid(c)).astype(_BF16)
    xn = _layernorm(x_v[...].astype(_F32))
    st.advance_to(n_mq)
    for t in range(6):
        w = wm_v[:, :, :, t * D:(t + 1) * D].reshape(D, D)
        mod_v[t] = jnp.dot(sc, w, preferred_element_type=_F32)
        st.advance(2)
    h1 = (xn * (1.0 + mod_v[1]) + mod_v[0]).astype(_BF16)
    hq = 4
    for h0 in range(0, H, hq):
        w = wq_v[:, :, :, h0 * Dh:(h0 + hq) * Dh].reshape(D, hq * Dh)
        q = jnp.dot(h1, w, preferred_element_type=_F32) * (Dh ** -0.5)
        for h in range(h0, h0 + hq):
            q_v[h] = q[:, (h - h0) * Dh:(h - h0 + 1) * Dh]
        st.advance(2)
    st.advance_to(len(pro))

    row = jax.lax.broadcasted_iota(jnp.int32, (B, _CK), 0)
    hps = wo_v.shape[2] // Dh

    def project(i, a_out):
        for t in range(2):
            h = i + t * H2
            ro = (h % hps) * Dh
            if not isinstance(i, int):
                ro = pl.multiple_of(ro, Dh)
            w = wo_v[h // (2 * hps), (h // hps) % 2, pl.ds(ro, Dh), :]
            a_out = a_out + jnp.dot(att_v[t].astype(_BF16), w, preferred_element_type=_F32)
        return a_out

    def head_rows(buf, c, t, b0=0, nb=None):
        nb = B if nb is None else nb
        return jnp.concatenate([buf[c, 2 * b + t] for b in range(b0, b0 + nb)], axis=0)

    def step(i, nxt, a_out):
        st = _Stream(step_pieces(i), nxt, look)
        qs = [q_v[i + t * H2].astype(_BF16) for t in range(2)]
        s = [[None] * nch, [None] * nch]

        def bursts(n):
            nb = 2 * B // n
            return [(k * nb // B, (k * nb) % B, min(nb, B)) for k in range(n)]

        def scores(c, t, b0, nb):
            sp = jax.lax.dot_general(qs[t], head_rows(kbuf, c, t, b0, nb), _NT,
                                     preferred_element_type=_F32)
            for r in range(nb):
                blk = sp[:, r * _CK:(r + 1) * _CK]
                s[t][c] = blk if s[t][c] is None else jnp.where(row == b0 + r, blk, s[t][c])

        st.advance(2)
        a_out = project(jnp.maximum(i - 1, 0) if not isinstance(i, int) else i - 1, a_out)
        for c in range(nch):
            for off, (t, b0, nb) in zip(koffs, bursts(len(koffs))):
                st.advance_to((c + 1) * ppc + off)
                scores(c, t, b0, nb)
        st.advance(1)
        p, l = [], []
        for t in range(2):
            m = jnp.max(functools.reduce(jnp.maximum, s[t]), axis=-1, keepdims=True)
            p.append([jnp.exp(v - m) for v in s[t]])
            l.append(jnp.sum(functools.reduce(jnp.add, p[t]), axis=-1, keepdims=True))
        for c in range(nch):
            for off, (t, b0, nb) in zip(voffs, bursts(len(voffs))):
                st.advance_to(max(st.pos, min((nch + c + 1) * ppc + off, 2 * nch * ppc)))
                pd = jnp.concatenate(
                    [jnp.where(row == r, p[t][c], 0.0) for r in range(b0, b0 + nb)],
                    axis=-1).astype(_BF16)
                o = jnp.dot(pd, head_rows(vbuf, c, t, b0, nb), preferred_element_type=_F32)
                if c > 0 or b0 > 0:
                    o = o + att_v[t]
                att_v[t] = o / l[t] if c == nch - 1 and b0 + nb == B else o
        return a_out

    a_out = jax.lax.fori_loop(0, n_steps - 1, lambda i, acc: step(i, step_pieces(i + 1), acc),
                              jnp.zeros((B, D), _F32))
    a_out = step(n_steps - 1, epi, a_out)

    st = _Stream(epi, [], look)
    st.advance(1)
    a_out = project(n_steps - 1, a_out)
    x1 = x_v[...].astype(_F32) + mod_v[2] * a_out
    st.advance(1)
    h2 = (_layernorm(x1) * (1.0 + mod_v[4]) + mod_v[3]).astype(_BF16)
    acc = jnp.zeros((B, D), _F32)
    hh = []
    nd = 0
    while nd < len(tiles):
        if len(hh) < len(tiles):
            pos = ready[(1, tiles[len(hh)][1] - 1)]
        else:
            pos = ready[(2, tiles[nd][1] - 1)]
        st.advance_to(max(pos, st.pos))
        have = len(hh)
        if have < len(tiles):
            lo, hi = tiles[have]
            sl = pl.ds(lo * _FC, (hi - lo) * _FC)
            g = jax.lax.dot_general(h2, wg_v[sl, :], _NT, preferred_element_type=_F32)
            u = jax.lax.dot_general(h2, wu_v[sl, :], _NT, preferred_element_type=_F32)
            hh.append((jax.nn.sigmoid(g) * u).astype(_BF16))
        while nd < have and ready[(2, tiles[nd][1] - 1)] <= st.pos:
            lo, hi = tiles[nd]
            acc = acc + jnp.dot(hh[nd], wd_v[pl.ds(lo * _FC, (hi - lo) * _FC), :],
                                preferred_element_type=_F32)
            nd += 1
    assert st.pos == len(epi)
    o_ref[...] = (x1 + mod_v[5] * acc).astype(o_ref.dtype)


def _forward(A_x, A_k_cache, A_v_cache, A_wq, A_wo, B_w_gate, B_w_up, B_w_down, c, w_mod,
             look=10, dlag=8, shift=8, runs=(2, 2, 2, 2, 3), koffs=(0, 3), voffs=(0, 3), nochecks=True):
    B, Sq, D = A_x.shape
    _, H, S, Dh = A_k_cache.shape
    F = B_w_down.shape[0]
    W = min(4096, max(256, S // 4))
    nch = W // _CK
    slab = lambda w: w.reshape(4, 2, w.shape[0] // 8, w.shape[1])
    wm, wq, wo = slab(w_mod), slab(A_wq), slab(A_wo)
    kv_shape = (2 * B, H // 2, S, Dh)
    any_spec = pl.BlockSpec(memory_space=pl.ANY)
    out = pl.pallas_call(
        functools.partial(_kernel, W=W, look=look, dlag=dlag, shift=shift, runs=tuple(runs), koffs=tuple(koffs), voffs=tuple(voffs)),
        in_specs=[any_spec] * 10,
        out_specs=pl.BlockSpec(memory_space=pltpu.VMEM),
        out_shape=jax.ShapeDtypeStruct((B, D), A_x.dtype),
        scratch_shapes=[
            pltpu.VMEM((B, D), _BF16),
            pltpu.VMEM((B, D), _BF16),
            pltpu.VMEM(wm.shape, _BF16),
            pltpu.VMEM(wq.shape, _BF16),
            pltpu.VMEM(wo.shape, _BF16),
            pltpu.VMEM((F, D), _BF16),
            pltpu.VMEM((F, D), _BF16),
            pltpu.VMEM((F, D), _BF16),
            pltpu.VMEM((nch, 2 * B, _CK, Dh), _BF16),
            pltpu.VMEM((nch, 2 * B, _CK, Dh), _BF16),
            pltpu.VMEM((6, B, D), _F32),
            pltpu.VMEM((H, B, Dh), _F32),
            pltpu.VMEM((2, B, Dh), _F32),
            pltpu.SemaphoreType.DMA((2 * nch,)),
        ],
        compiler_params=pltpu.CompilerParams(vmem_limit_bytes=64 * 1024 * 1024,
                                             disable_bounds_checks=nochecks,
                                             disable_semaphore_checks=nochecks),
    )(A_x.reshape(B, D), A_k_cache.reshape(kv_shape), A_v_cache.reshape(kv_shape), wq, wo,
      B_w_gate.T, B_w_up.T, B_w_down, c, wm)
    return out.reshape(B, Sq, D)


@jax.jit
def pallas_adaLN_cond__sliding_block_cached__glu_gated_glu__decode_kernel(
    A_x: jax.Array,
    A_k_cache: jax.Array,
    A_v_cache: jax.Array,
    A_wq: jax.Array,
    A_wo: jax.Array,
    B_x: jax.Array,
    B_w_gate: jax.Array,
    B_w_up: jax.Array,
    B_w_down: jax.Array,
    c: jax.Array,
    w_mod: jax.Array,
):
    del B_x
    return _forward(A_x, A_k_cache, A_v_cache, A_wq, A_wo, B_w_gate, B_w_up, B_w_down, c, w_mod)
```

```python
import functools

import jax
import jax.numpy as jnp
import jax.experimental.pallas as pl
import jax.experimental.pallas.tpu as pltpu

_NT = (((1,), (1,)), ((), ()))
_EPS = 1e-5
_F32 = jnp.float32
_BF16 = jnp.bfloat16
_CK = 128
_FC = 32
_TPC = 16
_SLABS = 8


def _layernorm(x):
    m = jnp.mean(x, axis=-1, keepdims=True)
    xc = x - m
    v = jnp.mean(xc * xc, axis=-1, keepdims=True)
    return xc * jax.lax.rsqrt(v + _EPS)


def _spans(total, n, off):
    out = [[((c - 1) * n + off, n, 0)] for c in range(total // n)]
    out[0] = [(total - n + off, n - off, 0)] + ([(0, off, n - off)] if off else [])
    return out


def _unit_groups(runs):
    n0 = len(runs)
    return [(pl.ds(g, 1), pl.ds(n0 + sum(runs[:g]), runs[g])) for g in range(n0)]


class _Piece:
    def __init__(self, parts, sem):
        self.parts, self.sem = parts, sem

    def start(self):
        for src, dst, prio in self.parts:
            pltpu.make_async_copy(src, dst, self.sem).start(priority=prio)

    def wait(self):
        for src, dst, _ in self.parts:
            pltpu.make_async_copy(src, dst, self.sem).wait()


class _Stream:
    def __init__(self, cur, nxt, look):
        self.cur, self.all, self.look, self.pos = cur, cur + nxt, look, 0

    def advance(self, n=1):
        for _ in range(n):
            self.cur[self.pos].wait()
            if self.pos + self.look < len(self.all):
                self.all[self.pos + self.look].start()
            self.pos += 1

    def advance_to(self, pos):
        self.advance(min(pos, len(self.cur)) - self.pos)


def _kernel(x_hbm, k_hbm, v_hbm, wq_hbm, wo_hbm, wg_hbm, wu_hbm, wd_hbm, c_hbm, wm_hbm,
            o_ref,
            x_v, c_v, wm_v, wq_v, wo_v, wg_v, wu_v, wd_v, kbuf, vbuf, mod_v, q_v, att_v, sems,
            *, W, look, kv_shift, kv_runs, lag, w_shifts, w_runs, dlag):
    B, D = x_v.shape
    nu, H2, S, Dh = k_hbm.shape
    F = wd_v.shape[0]
    nsem = sems.shape[0]
    nch = W // _CK

    counter = [0]

    def next_sem():
        counter[0] += 1
        return sems.at[(counter[0] - 1) % nsem]

    def weight_parts(src, dst, off):
        return [[(src.at[us, pl.ds(lo, n)], dst.at[us, pl.ds(lo, n)], prio)
                 for lo, n, _ in span for prio, us in enumerate(units)]
                for span in _spans(src.shape[1], _TPC, off) for units in _unit_groups(w_runs)]

    pro = [_Piece([(c_hbm, c_v, 0)], next_sem()), _Piece([(x_hbm, x_v, 0)], next_sem())]
    pm, pq = weight_parts(wm_hbm, wm_v, w_shifts[0]), weight_parts(wq_hbm, wq_v, w_shifts[1])
    keyed = [((i + 0.5) / len(pm), p) for i, p in enumerate(pm)]
    keyed += [((i + 0.51) / len(pq), p) for i, p in enumerate(pq)]
    pro += [_Piece(p, next_sem()) for _, p in sorted(keyed, key=lambda kp: kp[0])]
    n_mq = len(pro)
    pro += [_Piece(p, next_sem()) for p in weight_parts(wo_hbm, wo_v, w_shifts[2])]

    ppc = len(kv_runs)
    assert ppc + sum(kv_runs) == nu and len(w_runs) + sum(w_runs) == _SLABS
    assert (2 * nch * ppc) % nsem == 0 and look < nsem and lag < ppc
    sem0 = counter[0]

    def step_pieces(i):
        out = []
        for src, dst in ((k_hbm, kbuf), (v_hbm, vbuf)):
            for c, span in enumerate(_spans(W, _CK, kv_shift)):
                for units in _unit_groups(kv_runs):
                    parts = [(src.at[us, i, pl.ds(S - W + lo, n)],
                              dst.at[c, us, pl.ds(off, n)], prio)
                             for lo, n, off in span for prio, us in enumerate(units)]
                    out.append(_Piece(parts, sems.at[(sem0 + len(out)) % nsem]))
        return out

    nfc = F // _FC
    perm = [(s % 2) * ((nfc + 1) // 2) + s // 2 for s in range(nfc)]
    spt = 128 // _FC
    bounds = ([0] if nfc % spt else []) + list(range(nfc % spt, nfc + 1, spt))
    tiles = list(zip(bounds[:-1], bounds[1:]))
    seq = []
    for s in range(nfc + dlag):
        seq += [(0, s), (1, s)] if s < nfc else []
        seq += [(2, s - dlag)] if s >= dlag else []
    groups = [seq[max(e - spt, 0):e] for e in range(len(seq), 0, -spt)][::-1]
    epi, ready = [], {}
    ffn_refs = ((wg_hbm, wg_v), (wu_hbm, wu_v), (wd_hbm, wd_v))
    for j, grp in enumerate(groups):
        parts = []
        for t, (a, s) in enumerate(grp):
            src, dst = ffn_refs[a]
            prio = 0 if t == 0 and j < len(groups) - 1 else 1
            parts.append((src.at[pl.ds(perm[s] * _FC, _FC)], dst.at[pl.ds(s * _FC, _FC)], prio))
            ready[(a, s)] = j + 1
        epi.append(_Piece(parts, next_sem()))

    def columns(w_v, c0, nc):
        ns, nt = w_v.shape[:2]
        tpr = ns * nt * 8 // D
        t = jnp.stack([w_v[si, pl.ds(r * tpr + c0, nc)]
                       for si in range(ns) for r in range(nt // tpr)])
        return [t[:, j].reshape(D, 128) for j in range(nc)]

    st = _Stream(pro, step_pieces(0), look)
    for p in pro[:look]:
        p.start()
    att_v[...] = jnp.zeros(att_v.shape, _F32)
    st.advance(2)
    c = c_v[...].astype(_F32)
    sc = (c * jax.nn.sigmoid(c)).astype(_BF16)
    xn = _layernorm(x_v[...].astype(_F32))
    st.advance_to(n_mq)
    for t in range(6):
        for j, w in enumerate(columns(wm_v, t * D // 128, D // 128)):
            mod_v[t, :, j * 128:(j + 1) * 128] = jnp.dot(sc, w, preferred_element_type=_F32)
        st.advance(len(w_runs))
    h1 = (xn * (1.0 + mod_v[1]) + mod_v[0]).astype(_BF16)
    for h0 in range(0, 2 * H2, 4):
        for h, w in enumerate(columns(wq_v, h0, 4), h0):
            q_v[h] = jnp.dot(h1, w, preferred_element_type=_F32) * (Dh ** -0.5)
        st.advance(len(w_runs))
    st.advance_to(len(pro))

    row = jax.lax.broadcasted_iota(jnp.int32, (B, _CK), 0)
    tph = Dh * D // (8 * 128)
    hps = wo_v.shape[1] // tph

    def project(i, a_out):
        for t in range(2):
            h = i + t * H2
            w = wo_v[h // hps, pl.ds((h % hps) * tph, tph)].reshape(Dh // 8, D // 128, 8, 128)
            att = att_v[t].astype(_BF16)
            a_out = a_out + jnp.concatenate(
                [jnp.dot(att, w[:, j].reshape(Dh, 128), preferred_element_type=_F32)
                 for j in range(D // 128)], axis=-1)
        return a_out

    def head_rows(buf, c, t):
        return jnp.concatenate([buf[c, 2 * b + t] for b in range(B)], axis=0)

    def step(i, nxt, a_out):
        st = _Stream(step_pieces(i), nxt, look)
        st.advance(2)
        a_out = project(i - 1 if isinstance(i, int) else jnp.maximum(i - 1, 0), a_out)
        s = [[], []]
        for c in range(nch):
            for t in range(2):
                st.advance_to((c + 1) * ppc + t * lag)
                sp = jax.lax.dot_general(q_v[i + t * H2].astype(_BF16), head_rows(kbuf, c, t),
                                         _NT, preferred_element_type=_F32)
                sd = sp[:, :_CK]
                for b in range(1, B):
                    sd = jnp.where(row == b, sp[:, b * _CK:(b + 1) * _CK], sd)
                s[t].append(sd)
        st.advance(1)
        p, l = [], []
        for t in range(2):
            m = jnp.max(functools.reduce(jnp.maximum, s[t]), axis=-1, keepdims=True)
            p.append([jnp.exp(v - m) for v in s[t]])
            l.append(jnp.sum(functools.reduce(jnp.add, p[t]), axis=-1, keepdims=True))
        for c in range(nch):
            for t in range(2):
                st.advance_to((nch + c + 1) * ppc + t * lag)
                pd = jnp.concatenate([jnp.where(row == b, p[t][c], 0.0) for b in range(B)],
                                     axis=-1).astype(_BF16)
                o = jnp.dot(pd, head_rows(vbuf, c, t), preferred_element_type=_F32)
                if c > 0:
                    o = o + att_v[t]
                att_v[t] = o / l[t] if c == nch - 1 else o
        return a_out

    a_out = jax.lax.fori_loop(0, H2 - 1, lambda i, acc: step(i, step_pieces(i + 1), acc),
                              jnp.zeros((B, D), _F32))
    a_out = step(H2 - 1, epi, a_out)

    st = _Stream(epi, [], look)
    st.advance(1)
    x1 = x_v[...].astype(_F32) + mod_v[2] * project(H2 - 1, a_out)
    st.advance(1)
    h2 = (_layernorm(x1) * (1.0 + mod_v[4]) + mod_v[3]).astype(_BF16)
    acc = jnp.zeros((B, D), _F32)
    hh = []
    nd = 0
    while nd < len(tiles):
        have = len(hh)
        key = (1, tiles[have][1] - 1) if have < len(tiles) else (2, tiles[nd][1] - 1)
        st.advance_to(max(ready[key], st.pos))
        if have < len(tiles):
            lo, hi = tiles[have]
            sl = pl.ds(lo * _FC, (hi - lo) * _FC)
            g = jax.lax.dot_general(h2, wg_v[sl, :], _NT, preferred_element_type=_F32)
            u = jax.lax.dot_general(h2, wu_v[sl, :], _NT, preferred_element_type=_F32)
            hh.append((jax.nn.sigmoid(g) * u).astype(_BF16))
        while nd < have and ready[(2, tiles[nd][1] - 1)] <= st.pos:
            lo, hi = tiles[nd]
            acc = acc + jnp.dot(hh[nd], wd_v[pl.ds(lo * _FC, (hi - lo) * _FC), :],
                                preferred_element_type=_F32)
            nd += 1
    assert st.pos == len(epi)
    o_ref[...] = (x1 + mod_v[5] * acc).astype(o_ref.dtype)


def _forward(A_x, A_k_cache, A_v_cache, A_wq, A_wo, B_w_gate, B_w_up, B_w_down, c, w_mod,
             look=11, kv_shift=8, kv_runs=(2, 2, 2, 2, 3), lag=3, w_shifts=(9, 1, 1),
             w_runs=(2, 2, 1), dlag=8, nochecks=True):
    B, Sq, D = A_x.shape
    _, H, S, Dh = A_k_cache.shape
    F = B_w_down.shape[0]
    W = min(4096, max(256, S // 4))
    nch = W // _CK

    def tiled(w):
        r, cdim = w.shape
        t = w.reshape(r // 8, 8, cdim // 128, 128).transpose(0, 2, 1, 3)
        return t.reshape(_SLABS, -1, 8, 128)

    wm, wq, wo = tiled(w_mod), tiled(A_wq), tiled(A_wo)
    kv_shape = (2 * B, H // 2, S, Dh)
    out = pl.pallas_call(
        functools.partial(_kernel, W=W, look=look, kv_shift=kv_shift, kv_runs=tuple(kv_runs),
                          lag=lag, w_shifts=tuple(w_shifts), w_runs=tuple(w_runs), dlag=dlag),
        in_specs=[pl.BlockSpec(memory_space=pl.ANY)] * 10,
        out_specs=pl.BlockSpec(memory_space=pltpu.VMEM),
        out_shape=jax.ShapeDtypeStruct((B, D), A_x.dtype),
        scratch_shapes=[
            pltpu.VMEM((B, D), _BF16),
            pltpu.VMEM((B, D), _BF16),
            pltpu.VMEM(wm.shape, _BF16),
            pltpu.VMEM(wq.shape, _BF16),
            pltpu.VMEM(wo.shape, _BF16),
            pltpu.VMEM((F, D), _BF16),
            pltpu.VMEM((F, D), _BF16),
            pltpu.VMEM((F, D), _BF16),
            pltpu.VMEM((nch, 2 * B, _CK, Dh), _BF16),
            pltpu.VMEM((nch, 2 * B, _CK, Dh), _BF16),
            pltpu.VMEM((6, B, D), _F32),
            pltpu.VMEM((H, B, Dh), _F32),
            pltpu.VMEM((2, B, Dh), _F32),
            pltpu.SemaphoreType.DMA((2 * nch,)),
        ],
        compiler_params=pltpu.CompilerParams(vmem_limit_bytes=64 * 1024 * 1024,
                                             disable_bounds_checks=nochecks,
                                             disable_semaphore_checks=nochecks),
    )(A_x.reshape(B, D), A_k_cache.reshape(kv_shape), A_v_cache.reshape(kv_shape), wq, wo,
      B_w_gate.T, B_w_up.T, B_w_down, c, wm)
    return out.reshape(B, Sq, D)


@jax.jit
def pallas_adaLN_cond__sliding_block_cached__glu_gated_glu__decode_kernel(
    A_x: jax.Array,
    A_k_cache: jax.Array,
    A_v_cache: jax.Array,
    A_wq: jax.Array,
    A_wo: jax.Array,
    B_x: jax.Array,
    B_w_gate: jax.Array,
    B_w_up: jax.Array,
    B_w_down: jax.Array,
    c: jax.Array,
    w_mod: jax.Array,
):
    del B_x
    return _forward(A_x, A_k_cache, A_v_cache, A_wq, A_wo, B_w_gate, B_w_up, B_w_down, c, w_mod)
```

```python
import functools

import jax
import jax.numpy as jnp
import jax.experimental.pallas as pl
import jax.experimental.pallas.tpu as pltpu

_NT = (((1,), (1,)), ((), ()))
_EPS = 1e-5
_F32 = jnp.float32
_BF16 = jnp.bfloat16
_CK = 128
_FC = 32
_TPC = 16
_SLABS = 8


def _layernorm(x):
    m = jnp.mean(x, axis=-1, keepdims=True)
    xc = x - m
    v = jnp.mean(xc * xc, axis=-1, keepdims=True)
    return xc * jax.lax.rsqrt(v + _EPS)


def _spans(total, n, off):
    out = [[((c - 1) * n + off, n, 0)] for c in range(total // n)]
    out[0] = [(total - n + off, n - off, 0)] + ([(0, off, n - off)] if off else [])
    return out


def _unit_groups(runs):
    n0 = len(runs)
    return [(pl.ds(g, 1), pl.ds(n0 + sum(runs[:g]), runs[g])) for g in range(n0)]


class _Piece:
    def __init__(self, parts, sem):
        self.parts, self.sem = parts, sem

    def start(self):
        for src, dst, prio in self.parts:
            pltpu.make_async_copy(src, dst, self.sem).start(priority=prio)

    def wait(self):
        for src, dst, _ in self.parts:
            pltpu.make_async_copy(src, dst, self.sem).wait()


class _Stream:
    def __init__(self, cur, nxt, look):
        self.cur, self.all, self.look, self.pos = cur, cur + nxt, look, 0

    def advance(self, n=1):
        for _ in range(n):
            self.cur[self.pos].wait()
            if self.pos + self.look < len(self.all):
                self.all[self.pos + self.look].start()
            self.pos += 1

    def advance_to(self, pos):
        self.advance(min(pos, len(self.cur)) - self.pos)


def _kernel(x_hbm, k_hbm, v_hbm, wq_hbm, wo_hbm, wg_hbm, wu_hbm, wd_hbm, c_hbm, wm_hbm,
            o_ref,
            x_v, c_v, wm_v, wq_v, wo_v, wg_v, wu_v, wd_v, kbuf, vbuf, mod_v, q_v, att_v, sems,
            *, W, look, kv_shift, kv_runs, lag, w_shifts, w_runs, dlag):
    B, D = x_v.shape
    nu, H2, S, Dh = k_hbm.shape
    F = wd_v.shape[0]
    nsem = sems.shape[0]
    nch = W // _CK

    counter = [0]

    def next_sem():
        counter[0] += 1
        return sems.at[(counter[0] - 1) % nsem]

    def weight_parts(src, dst, off):
        return [[(src.at[us, pl.ds(lo, n)], dst.at[us, pl.ds(lo, n)], prio)
                 for lo, n, _ in span for prio, us in enumerate(units)]
                for span in _spans(src.shape[1], _TPC, off) for units in _unit_groups(w_runs)]

    pro = [_Piece([(c_hbm, c_v, 0)], next_sem()), _Piece([(x_hbm, x_v, 0)], next_sem())]
    pm, pq = weight_parts(wm_hbm, wm_v, w_shifts[0]), weight_parts(wq_hbm, wq_v, w_shifts[1])
    keyed = [((i + 0.5) / len(pm), p) for i, p in enumerate(pm)]
    keyed += [((i + 0.51) / len(pq), p) for i, p in enumerate(pq)]
    pro += [_Piece(p, next_sem()) for _, p in sorted(keyed, key=lambda kp: kp[0])]
    n_mq = len(pro)
    pro += [_Piece(p, next_sem()) for p in weight_parts(wo_hbm, wo_v, w_shifts[2])]

    ppc = len(kv_runs)
    assert ppc + sum(kv_runs) == nu and len(w_runs) + sum(w_runs) == _SLABS
    assert (2 * nch * ppc) % nsem == 0 and look < nsem and lag < ppc
    sem0 = counter[0]

    def step_pieces(i):
        out = []
        for src, dst in ((k_hbm, kbuf), (v_hbm, vbuf)):
            for c, span in enumerate(_spans(W, _CK, kv_shift)):
                for units in _unit_groups(kv_runs):
                    parts = [(src.at[us, i, pl.ds(S - W + lo, n)],
                              dst.at[c, us, pl.ds(off, n)], prio)
                             for lo, n, off in span for prio, us in enumerate(units)]
                    out.append(_Piece(parts, sems.at[(sem0 + len(out)) % nsem]))
        return out

    nfc = F // _FC
    perm = [(s % 2) * ((nfc + 1) // 2) + s // 2 for s in range(nfc)]
    spt = 128 // _FC
    bounds = ([0] if nfc % spt else []) + list(range(nfc % spt, nfc + 1, spt))
    tiles = list(zip(bounds[:-1], bounds[1:]))
    seq = []
    for s in range(nfc + dlag):
        seq += [(0, s), (1, s)] if s < nfc else []
        seq += [(2, s - dlag)] if s >= dlag else []
    groups = [seq[max(e - spt, 0):e] for e in range(len(seq), 0, -spt)][::-1]
    epi, ready = [], {}
    ffn_refs = ((wg_hbm, wg_v), (wu_hbm, wu_v), (wd_hbm, wd_v))
    for j, grp in enumerate(groups):
        parts = []
        for t, (a, s) in enumerate(grp):
            src, dst = ffn_refs[a]
            prio = 0 if t == 0 and j < len(groups) - 1 else 1
            parts.append((src.at[pl.ds(perm[s] * _FC, _FC)], dst.at[pl.ds(s * _FC, _FC)], prio))
            ready[(a, s)] = j + 1
        epi.append(_Piece(parts, next_sem()))

    def columns(w_v, c0, nc):
        t = w_v[...].reshape(D // 8, -1, 8, 128)
        return [t[:, j].reshape(D, 128) for j in range(c0, c0 + nc)]

    st = _Stream(pro, step_pieces(0), look)
    for p in pro[:look]:
        p.start()
    att_v[...] = jnp.zeros(att_v.shape, _F32)
    st.advance(2)
    c = c_v[...].astype(_F32)
    sc = (c * jax.nn.sigmoid(c)).astype(_BF16)
    xn = _layernorm(x_v[...].astype(_F32))
    st.advance_to(n_mq)
    for t in range(6):
        for j, w in enumerate(columns(wm_v, t * D // 128, D // 128)):
            mod_v[t, :, j * 128:(j + 1) * 128] = jnp.dot(sc, w, preferred_element_type=_F32)
        st.advance(len(w_runs))
    h1 = (xn * (1.0 + mod_v[1]) + mod_v[0]).astype(_BF16)
    for h0 in range(0, 2 * H2, 4):
        for h, w in enumerate(columns(wq_v, h0, 4), h0):
            q_v[h] = jnp.dot(h1, w, preferred_element_type=_F32) * (Dh ** -0.5)
        st.advance(len(w_runs))
    st.advance_to(len(pro))

    row = jax.lax.broadcasted_iota(jnp.int32, (B, _CK), 0)
    tph = Dh * D // (8 * 128)
    hps = wo_v.shape[1] // tph

    def project(i, a_out):
        for t in range(2):
            h = i + t * H2
            w = wo_v[h // hps, pl.ds((h % hps) * tph, tph)].reshape(Dh // 8, D // 128, 8, 128)
            att = att_v[t].astype(_BF16)
            a_out = a_out + jnp.concatenate(
                [jnp.dot(att, w[:, j].reshape(Dh, 128), preferred_element_type=_F32)
                 for j in range(D // 128)], axis=-1)
        return a_out

    def head_rows(buf, c, t):
        return buf[c].reshape(B, 2, _CK, Dh)[:, t].reshape(B * _CK, Dh)

    def step(i, nxt, a_out):
        st = _Stream(step_pieces(i), nxt, look)
        st.advance(2)
        a_out = project(i - 1 if isinstance(i, int) else jnp.maximum(i - 1, 0), a_out)
        s = [[], []]
        for c in range(nch):
            for t in range(2):
                st.advance_to((c + 1) * ppc + t * lag)
                sp = jax.lax.dot_general(q_v[i + t * H2].astype(_BF16), head_rows(kbuf, c, t),
                                         _NT, preferred_element_type=_F32)
                sd = sp[:, :_CK]
                for b in range(1, B):
                    sd = jnp.where(row == b, sp[:, b * _CK:(b + 1) * _CK], sd)
                s[t].append(sd)
        st.advance(1)
        p, l = [], []
        for t in range(2):
            m = jnp.max(functools.reduce(jnp.maximum, s[t]), axis=-1, keepdims=True)
            p.append([jnp.exp(v - m) for v in s[t]])
            l.append(jnp.sum(functools.reduce(jnp.add, p[t]), axis=-1, keepdims=True))
        for c in range(nch):
            for t in range(2):
                st.advance_to((nch + c + 1) * ppc + t * lag)
                pd = jnp.concatenate([jnp.where(row == b, p[t][c], 0.0) for b in range(B)],
                                     axis=-1).astype(_BF16)
                o = jnp.dot(pd, head_rows(vbuf, c, t), preferred_element_type=_F32)
                if c > 0:
                    o = o + att_v[t]
                att_v[t] = o / l[t] if c == nch - 1 else o
        return a_out

    a_out = jax.lax.fori_loop(0, H2 - 1, lambda i, acc: step(i, step_pieces(i + 1), acc),
                              jnp.zeros((B, D), _F32))
    a_out = step(H2 - 1, epi, a_out)

    st = _Stream(epi, [], look)
    st.advance(1)
    x1 = x_v[...].astype(_F32) + mod_v[2] * project(H2 - 1, a_out)
    st.advance(1)
    h2 = (_layernorm(x1) * (1.0 + mod_v[4]) + mod_v[3]).astype(_BF16)
    acc = jnp.zeros((B, D), _F32)
    hh = []
    nd = 0
    while nd < len(tiles):
        have = len(hh)
        key = (1, tiles[have][1] - 1) if have < len(tiles) else (2, tiles[nd][1] - 1)
        st.advance_to(max(ready[key], st.pos))
        if have < len(tiles):
            lo, hi = tiles[have]
            sl = pl.ds(lo * _FC, (hi - lo) * _FC)
            g = jax.lax.dot_general(h2, wg_v[sl, :], _NT, preferred_element_type=_F32)
            u = jax.lax.dot_general(h2, wu_v[sl, :], _NT, preferred_element_type=_F32)
            hh.append((jax.nn.sigmoid(g) * u).astype(_BF16))
        while nd < have and ready[(2, tiles[nd][1] - 1)] <= st.pos:
            lo, hi = tiles[nd]
            acc = acc + jnp.dot(hh[nd], wd_v[pl.ds(lo * _FC, (hi - lo) * _FC), :],
                                preferred_element_type=_F32)
            nd += 1
    assert st.pos == len(epi)
    o_ref[...] = (x1 + mod_v[5] * acc).astype(o_ref.dtype)


def _forward(A_x, A_k_cache, A_v_cache, A_wq, A_wo, B_w_gate, B_w_up, B_w_down, c, w_mod,
             look=11, kv_shift=8, kv_runs=(2, 2, 2, 2, 3), lag=3, w_shifts=(9, 1, 1),
             w_runs=(2, 2, 1), dlag=8, nochecks=True):
    B, Sq, D = A_x.shape
    _, H, S, Dh = A_k_cache.shape
    F = B_w_down.shape[0]
    W = min(4096, max(256, S // 4))
    nch = W // _CK

    def tiled(w):
        r, cdim = w.shape
        t = w.reshape(r // 8, 8, cdim // 128, 128).transpose(0, 2, 1, 3)
        return t.reshape(_SLABS, -1, 8, 128)

    wm, wq, wo = tiled(w_mod), tiled(A_wq), tiled(A_wo)
    kv_shape = (2 * B, H // 2, S, Dh)
    out = pl.pallas_call(
        functools.partial(_kernel, W=W, look=look, kv_shift=kv_shift, kv_runs=tuple(kv_runs),
                          lag=lag, w_shifts=tuple(w_shifts), w_runs=tuple(w_runs), dlag=dlag),
        in_specs=[pl.BlockSpec(memory_space=pl.ANY)] * 10,
        out_specs=pl.BlockSpec(memory_space=pltpu.VMEM),
        out_shape=jax.ShapeDtypeStruct((B, D), A_x.dtype),
        scratch_shapes=[
            pltpu.VMEM((B, D), _BF16),
            pltpu.VMEM((B, D), _BF16),
            pltpu.VMEM(wm.shape, _BF16),
            pltpu.VMEM(wq.shape, _BF16),
            pltpu.VMEM(wo.shape, _BF16),
            pltpu.VMEM((F, D), _BF16),
            pltpu.VMEM((F, D), _BF16),
            pltpu.VMEM((F, D), _BF16),
            pltpu.VMEM((nch, 2 * B, _CK, Dh), _BF16),
            pltpu.VMEM((nch, 2 * B, _CK, Dh), _BF16),
            pltpu.VMEM((6, B, D), _F32),
            pltpu.VMEM((H, B, Dh), _F32),
            pltpu.VMEM((2, B, Dh), _F32),
            pltpu.SemaphoreType.DMA((2 * nch,)),
        ],
        compiler_params=pltpu.CompilerParams(vmem_limit_bytes=64 * 1024 * 1024,
                                             disable_bounds_checks=nochecks,
                                             disable_semaphore_checks=nochecks),
    )(A_x.reshape(B, D), A_k_cache.reshape(kv_shape), A_v_cache.reshape(kv_shape), wq, wo,
      B_w_gate.T, B_w_up.T, B_w_down, c, wm)
    return out.reshape(B, Sq, D)


@jax.jit
def pallas_adaLN_cond__sliding_block_cached__glu_gated_glu__decode_kernel(
    A_x: jax.Array,
    A_k_cache: jax.Array,
    A_v_cache: jax.Array,
    A_wq: jax.Array,
    A_wo: jax.Array,
    B_x: jax.Array,
    B_w_gate: jax.Array,
    B_w_up: jax.Array,
    B_w_down: jax.Array,
    c: jax.Array,
    w_mod: jax.Array,
):
    del B_x
    return _forward(A_x, A_k_cache, A_v_cache, A_wq, A_wo, B_w_gate, B_w_up, B_w_down, c, w_mod)
```

```python
import functools

import jax
import jax.numpy as jnp
import jax.experimental.pallas as pl
import jax.experimental.pallas.tpu as pltpu

_NT = (((1,), (1,)), ((), ()))
_EPS = 1e-5
_F32 = jnp.float32
_BF16 = jnp.bfloat16
_CK = 128
_FC = 32
_TPC = 16
_SLABS = 8


def _layernorm(x):
    m = jnp.mean(x, axis=-1, keepdims=True)
    xc = x - m
    v = jnp.mean(xc * xc, axis=-1, keepdims=True)
    return xc * jax.lax.rsqrt(v + _EPS)


def _spans(total, n, off):
    out = [[((c - 1) * n + off, n, 0)] for c in range(total // n)]
    out[0] = [(total - n + off, n - off, 0)] + ([(0, off, n - off)] if off else [])
    return out


def _unit_groups(runs):
    n0 = len(runs)
    return [(pl.ds(g, 1), pl.ds(n0 + sum(runs[:g]), runs[g])) for g in range(n0)]


class _Piece:
    def __init__(self, parts, sem):
        self.parts, self.sem = parts, sem

    def start(self, only=None):
        for src, dst, prio in self.parts:
            if only is None or prio == only:
                pltpu.make_async_copy(src, dst, self.sem).start(priority=prio)

    def wait(self):
        for src, dst, _ in self.parts:
            pltpu.make_async_copy(src, dst, self.sem).wait()


class _Stream:
    def __init__(self, cur, nxt, look):
        self.cur, self.all, self.look, self.pos = cur, cur + nxt, look, 0

    def advance(self, n=1):
        for _ in range(n):
            self.cur[self.pos].wait()
            if self.pos + self.look < len(self.all):
                self.all[self.pos + self.look].start()
            self.pos += 1

    def advance_to(self, pos):
        self.advance(min(pos, len(self.cur)) - self.pos)


def _kernel(x_hbm, k_hbm, v_hbm, wq_hbm, wo_hbm, wg_hbm, wu_hbm, wd_hbm, c_hbm, wm_hbm,
            o_ref,
            x_v, c_v, wm_v, wq_v, wo_v, wg_v, wu_v, wd_v, kbuf, vbuf, mod_v, q_v, att_v, sems,
            *, W, look, kv_shift, kv_runs, lag, w_shifts, w_runs, dlag, spin):
    B, D = x_v.shape
    nu, H2, S, Dh = k_hbm.shape
    F = wd_v.shape[0]
    nsem = sems.shape[0]
    nch = W // _CK

    counter = [0]

    def next_sem():
        counter[0] += 1
        return sems.at[(counter[0] - 1) % nsem]

    def weight_parts(src, dst, off):
        return [[(src.at[us, pl.ds(lo, n)], dst.at[us, pl.ds(lo, n)], prio)
                 for lo, n, _ in span for prio, us in enumerate(units)]
                for span in _spans(src.shape[1], _TPC, off) for units in _unit_groups(w_runs)]

    pro = [_Piece([(c_hbm, c_v, 0)], next_sem()), _Piece([(x_hbm, x_v, 0)], next_sem())]
    pm, pq = weight_parts(wm_hbm, wm_v, w_shifts[0]), weight_parts(wq_hbm, wq_v, w_shifts[1])
    keyed = [((i + 0.5) / len(pm), p) for i, p in enumerate(pm)]
    keyed += [((i + 0.51) / len(pq), p) for i, p in enumerate(pq)]
    pro += [_Piece(p, next_sem()) for _, p in sorted(keyed, key=lambda kp: kp[0])]
    n_mq = len(pro)
    pro += [_Piece(p, next_sem()) for p in weight_parts(wo_hbm, wo_v, w_shifts[2])]

    ppc = len(kv_runs)
    assert ppc + sum(kv_runs) == nu and len(w_runs) + sum(w_runs) == _SLABS
    assert (2 * nch * ppc) % nsem == 0 and look < nsem and lag < ppc
    sem0 = counter[0]

    def step_pieces(i):
        out = []
        for src, dst in ((k_hbm, kbuf), (v_hbm, vbuf)):
            for c, span in enumerate(_spans(W, _CK, kv_shift)):
                for units in _unit_groups(kv_runs):
                    parts = [(src.at[us, i, pl.ds(S - W + lo, n)],
                              dst.at[c, us, pl.ds(off, n)], prio)
                             for lo, n, off in span for prio, us in enumerate(units)]
                    out.append(_Piece(parts, sems.at[(sem0 + len(out)) % nsem]))
        return out

    nfc = F // _FC
    perm = [(s % 2) * ((nfc + 1) // 2) + s // 2 for s in range(nfc)]
    spt = 128 // _FC
    bounds = ([0] if nfc % spt else []) + list(range(nfc % spt, nfc + 1, spt))
    tiles = list(zip(bounds[:-1], bounds[1:]))
    seq = []
    for s in range(nfc + dlag):
        seq += [(0, s), (1, s)] if s < nfc else []
        seq += [(2, s - dlag)] if s >= dlag else []
    groups = [seq[max(e - spt, 0):e] for e in range(len(seq), 0, -spt)][::-1]
    epi, ready = [], {}
    ffn_refs = ((wg_hbm, wg_v), (wu_hbm, wu_v), (wd_hbm, wd_v))
    for j, grp in enumerate(groups):
        parts = []
        for t, (a, s) in enumerate(grp):
            src, dst = ffn_refs[a]
            prio = 0 if t == 0 and j < len(groups) - dlag // spt else 1
            parts.append((src.at[pl.ds(perm[s] * _FC, _FC)], dst.at[pl.ds(s * _FC, _FC)], prio))
            ready[(a, s)] = j + 1
        epi.append(_Piece(parts, next_sem()))

    def columns(w_v, c0, nc):
        t = w_v[...].reshape(D // 8, -1, 8, 128)
        return [t[:, j].reshape(D, 128) for j in range(c0, c0 + nc)]

    st = _Stream(pro, step_pieces(0), look)
    for p in pro[:look]:
        p.start(only=1)
    z = jnp.ones((B, Dh), _F32)
    for j, p in enumerate(pro[:look]):
        p.start(only=0)
        if 2 <= j < look - 1:
            z = jax.lax.fori_loop(0, spin, lambda _, v: v * 0.5, z)
    for t in range(2):
        att_v[t] = jnp.where(z < 2.0, 0.0, z)
    st.advance(2)
    c = c_v[...].astype(_F32)
    sc = (c * jax.nn.sigmoid(c)).astype(_BF16)
    xn = _layernorm(x_v[...].astype(_F32))
    st.advance_to(n_mq)
    for t in range(6):
        for j, w in enumerate(columns(wm_v, t * D // 128, D // 128)):
            mod_v[t, :, j * 128:(j + 1) * 128] = jnp.dot(sc, w, preferred_element_type=_F32)
        st.advance(len(w_runs))
    h1 = (xn * (1.0 + mod_v[1]) + mod_v[0]).astype(_BF16)
    for h0 in range(0, 2 * H2, 4):
        for h, w in enumerate(columns(wq_v, h0, 4), h0):
            q_v[h] = jnp.dot(h1, w, preferred_element_type=_F32) * (Dh ** -0.5)
        st.advance(len(w_runs))
    st.advance_to(len(pro))

    row = jax.lax.broadcasted_iota(jnp.int32, (B, _CK), 0)
    tph = Dh * D // (8 * 128)
    hps = wo_v.shape[1] // tph

    def project(i, a_out):
        for t in range(2):
            h = i + t * H2
            w = wo_v[h // hps, pl.ds((h % hps) * tph, tph)].reshape(Dh // 8, D // 128, 8, 128)
            att = att_v[t].astype(_BF16)
            a_out = a_out + jnp.concatenate(
                [jnp.dot(att, w[:, j].reshape(Dh, 128), preferred_element_type=_F32)
                 for j in range(D // 128)], axis=-1)
        return a_out

    def head_rows(buf, c, t):
        return buf[c].reshape(B, 2, _CK, Dh)[:, t].reshape(B * _CK, Dh)

    def step(i, nxt, a_out):
        st = _Stream(step_pieces(i), nxt, look)
        st.advance(2)
        a_out = project(i - 1 if isinstance(i, int) else jnp.maximum(i - 1, 0), a_out)
        s = [[], []]
        for c in range(nch):
            for t in range(2):
                st.advance_to((c + 1) * ppc + t * lag)
                sp = jax.lax.dot_general(q_v[i + t * H2].astype(_BF16), head_rows(kbuf, c, t),
                                         _NT, preferred_element_type=_F32)
                sd = sp[:, :_CK]
                for b in range(1, B):
                    sd = jnp.where(row == b, sp[:, b * _CK:(b + 1) * _CK], sd)
                s[t].append(sd)
        st.advance(1)
        p, l = [], []
        for t in range(2):
            m = jnp.max(functools.reduce(jnp.maximum, s[t]), axis=-1, keepdims=True)
            p.append([jnp.exp(v - m) for v in s[t]])
            l.append(jnp.sum(functools.reduce(jnp.add, p[t]), axis=-1, keepdims=True))
        for c in range(nch):
            for t in range(2):
                st.advance_to((nch + c + 1) * ppc + t * lag)
                pd = jnp.concatenate([jnp.where(row == b, p[t][c], 0.0) for b in range(B)],
                                     axis=-1).astype(_BF16)
                o = jnp.dot(pd, head_rows(vbuf, c, t), preferred_element_type=_F32)
                if c > 0:
                    o = o + att_v[t]
                att_v[t] = o / l[t] if c == nch - 1 else o
        return a_out

    a_out = jax.lax.fori_loop(0, H2 - 1, lambda i, acc: step(i, step_pieces(i + 1), acc),
                              jnp.zeros((B, D), _F32))
    a_out = step(H2 - 1, epi, a_out)

    st = _Stream(epi, [], look)
    st.advance(1)
    x1 = x_v[...].astype(_F32) + mod_v[2] * project(H2 - 1, a_out)
    st.advance(1)
    h2 = (_layernorm(x1) * (1.0 + mod_v[4]) + mod_v[3]).astype(_BF16)
    acc = jnp.zeros((B, D), _F32)
    hh = []
    nd = 0
    while nd < len(tiles):
        have = len(hh)
        key = (1, tiles[have][1] - 1) if have < len(tiles) else (2, tiles[nd][1] - 1)
        st.advance_to(max(ready[key], st.pos))
        if have < len(tiles):
            lo, hi = tiles[have]
            sl = pl.ds(lo * _FC, (hi - lo) * _FC)
            g = jax.lax.dot_general(h2, wg_v[sl, :], _NT, preferred_element_type=_F32)
            u = jax.lax.dot_general(h2, wu_v[sl, :], _NT, preferred_element_type=_F32)
            hh.append((jax.nn.sigmoid(g) * u).astype(_BF16))
        while nd < have and ready[(2, tiles[nd][1] - 1)] <= st.pos:
            lo, hi = tiles[nd]
            acc = acc + jnp.dot(hh[nd], wd_v[pl.ds(lo * _FC, (hi - lo) * _FC), :],
                                preferred_element_type=_F32)
            nd += 1
    assert st.pos == len(epi)
    o_ref[...] = (x1 + mod_v[5] * acc).astype(o_ref.dtype)


def _forward(A_x, A_k_cache, A_v_cache, A_wq, A_wo, B_w_gate, B_w_up, B_w_down, c, w_mod,
             look=11, kv_shift=8, kv_runs=(2, 2, 2, 2, 3), lag=3, w_shifts=(9, 1, 1),
             w_runs=(2, 2, 1), dlag=16, spin=13, nochecks=True):
    B, Sq, D = A_x.shape
    _, H, S, Dh = A_k_cache.shape
    F = B_w_down.shape[0]
    W = min(4096, max(256, S // 4))
    nch = W // _CK

    def tiled(w):
        r, cdim = w.shape
        t = w.reshape(r // 8, 8, cdim // 128, 128).transpose(0, 2, 1, 3)
        return t.reshape(_SLABS, -1, 8, 128)

    wm, wq, wo = tiled(w_mod), tiled(A_wq), tiled(A_wo)
    kv_shape = (2 * B, H // 2, S, Dh)
    out = pl.pallas_call(
        functools.partial(_kernel, W=W, look=look, kv_shift=kv_shift, kv_runs=tuple(kv_runs),
                          lag=lag, w_shifts=tuple(w_shifts), w_runs=tuple(w_runs), dlag=dlag,
                          spin=spin),
        in_specs=[pl.BlockSpec(memory_space=pl.ANY)] * 10,
        out_specs=pl.BlockSpec(memory_space=pltpu.VMEM),
        out_shape=jax.ShapeDtypeStruct((B, D), A_x.dtype),
        scratch_shapes=[
            pltpu.VMEM((B, D), _BF16),
            pltpu.VMEM((B, D), _BF16),
            pltpu.VMEM(wm.shape, _BF16),
            pltpu.VMEM(wq.shape, _BF16),
            pltpu.VMEM(wo.shape, _BF16),
            pltpu.VMEM((F, D), _BF16),
            pltpu.VMEM((F, D), _BF16),
            pltpu.VMEM((F, D), _BF16),
            pltpu.VMEM((nch, 2 * B, _CK, Dh), _BF16),
            pltpu.VMEM((nch, 2 * B, _CK, Dh), _BF16),
            pltpu.VMEM((6, B, D), _F32),
            pltpu.VMEM((H, B, Dh), _F32),
            pltpu.VMEM((2, B, Dh), _F32),
            pltpu.SemaphoreType.DMA((2 * nch,)),
        ],
        compiler_params=pltpu.CompilerParams(vmem_limit_bytes=64 * 1024 * 1024,
                                             disable_bounds_checks=nochecks,
                                             disable_semaphore_checks=nochecks),
    )(A_x.reshape(B, D), A_k_cache.reshape(kv_shape), A_v_cache.reshape(kv_shape), wq, wo,
      B_w_gate.T, B_w_up.T, B_w_down, c, wm)
    return out.reshape(B, Sq, D)


@jax.jit
def pallas_adaLN_cond__sliding_block_cached__glu_gated_glu__decode_kernel(
    A_x: jax.Array,
    A_k_cache: jax.Array,
    A_v_cache: jax.Array,
    A_wq: jax.Array,
    A_wo: jax.Array,
    B_x: jax.Array,
    B_w_gate: jax.Array,
    B_w_up: jax.Array,
    B_w_down: jax.Array,
    c: jax.Array,
    w_mod: jax.Array,
):
    del B_x
    return _forward(A_x, A_k_cache, A_v_cache, A_wq, A_wo, B_w_gate, B_w_up, B_w_down, c, w_mod)
```
